```python
import os as _os
_os.environ.setdefault('JAX_PLATFORMS', 'cpu')
import jax
import jax.numpy as jnp

def _softmax(x, axis=-1):
    return jax.nn.softmax(x, axis=axis)

def _gelu(x):
    return jax.nn.gelu(x, approximate=True)

def _silu(x):
    return jax.nn.silu(x)

def _sigmoid(x):
    return jax.nn.sigmoid(x)

def _layernorm(x, axis=-1, eps=1e-05):
    m = jnp.mean(x, axis=axis, keepdims=True)
    v = jnp.var(x, axis=axis, keepdims=True)
    return (x - m) / jnp.sqrt(v + eps)

def _scatter_add(tgt, idx, src, axis=0):
    return tgt.at[idx].add(src)

def _segment_sum(src, seg, n):
    return jax.ops.segment_sum(src, seg, n)

class _Rng:

    def __init__(self, key):
        self._k = key

    def _next(self):
        self._k, sub = jax.random.split(self._k)
        return sub

    def normal(self, shape):
        return jax.random.normal(self._next(), shape, dtype=jnp.bfloat16)

    def randint(self, lo, hi, shape):
        return jax.random.randint(self._next(), shape, lo, hi, dtype=jnp.int32)

    def uniform(self, shape, lo=0.0, hi=1.0):
        return jax.random.uniform(self._next(), shape, jnp.bfloat16, lo, hi)

    def permutation(self, n):
        return jax.random.permutation(self._next(), n)
kernel_name = 'adaLN_cond__grouped_kv_mqa__mixer_gmlp__prompt'

def setup_inputs():
    _rng = _Rng(jax.random.key(int.from_bytes(__import__("os").urandom(4), "little")))
    _w = lambda a: (lambda t: t.astype(jnp.bfloat16) if jnp.issubdtype(t.dtype, jnp.floating) else t)(jnp.asarray(a))

    def _A_setup():
        B, S, D, H = (1, 2048, 512, 32)
        Dh = D // H
        return {'x': _w((lambda *s: _rng.normal(s) * 0.05)(B, S, D)), 'wq': _w((lambda *s: _rng.normal(s) * 0.05)(D, H * Dh)), 'wk': _w((lambda *s: _rng.normal(s) * 0.05)(D, Dh)), 'wv': _w((lambda *s: _rng.normal(s) * 0.05)(D, Dh)), 'wo': _w((lambda *s: _rng.normal(s) * 0.05)(H * Dh, D))}
    _A_in = _A_setup()

    def _B_setup():
        B, S, D, F = (1, 2048, 512, 1792)
        Fh = F // 2
        return {'x': _w((lambda *s: _rng.normal(s) * 0.05)(B, S, D)), 'w_in': _w((lambda *s: _rng.normal(s) * 0.4)(D, 2 * Fh)), 'w_sp': _w(0.01 * (lambda *s: _rng.normal(s) * 0.4)(S, S)), 'b_sp': _w(1.0 + 0.01 * (lambda *s: _rng.normal(s) * 0.05)(S)), 'w_out': _w((lambda *s: _rng.normal(s) * 0.05)(Fh, D))}
    _B_in = _B_setup()
    return {'A_x': _A_in['x'], 'A_wq': _A_in['wq'], 'A_wk': _A_in['wk'], 'A_wv': _A_in['wv'], 'A_wo': _A_in['wo'], 'B_x': _B_in['x'], 'B_w_in': _B_in['w_in'], 'B_w_sp': _B_in['w_sp'], 'B_b_sp': _B_in['b_sp'], 'B_w_out': _B_in['w_out'], 'c': _w((lambda *s: _rng.normal(s) * 0.05)(1, 512) * 8.0), 'w_mod': _w((lambda *s: _rng.normal(s) * 0.05)(512, 6 * 512) * 512 ** (-0.5) * 8.0)}

def reference(A_x, A_wq, A_wk, A_wv, A_wo, B_x, B_w_in, B_w_sp, B_b_sp, B_w_out, c, w_mod):

    def _A_ref(x, wq, wk, wv, wo):
        B, S, D = x.shape
        H = 32
        Dh = D // H
        q = (lambda x, *d: x.transpose(*d))((x @ wq).reshape(B, S, H, Dh), 0, 2, 1, 3)
        k = x @ wk
        v = x @ wv
        scores = jnp.einsum('bhqd,bkd->bhqk', q, k) * Dh ** (-0.5)
        p = _softmax(scores, axis=-1)
        o = jnp.einsum('bhqk,bkd->bhqd', p, v)
        return (lambda x, *d: x.transpose(*d))(o, 0, 2, 1, 3).reshape(B, S, H * Dh) @ wo

    def _B_ref(x, w_in, w_sp, b_sp, w_out):
        B, S, D = x.shape
        F = w_in.shape[-1]
        Fh = F // 2
        z = _gelu(jnp.einsum('bsd,df->bsf', x, w_in))
        z1 = z[..., :Fh].copy()
        z2 = _layernorm(z[..., Fh:], axis=-1)
        g = jnp.einsum('ts,bsf->btf', w_sp, z2) + b_sp[None, :, None]
        return jnp.einsum('bsf,fd->bsd', z1 * g, w_out)
    x = A_x
    mod = (_silu(c) @ w_mod).reshape(c.shape[0], 6, 1, -1)
    sa, ca, ga, sb, cb, gb = (mod[:, 0].copy(), mod[:, 1].copy(), mod[:, 2].copy(), mod[:, 3].copy(), mod[:, 4].copy(), mod[:, 5].copy())
    h = _layernorm(x, axis=-1) * (1 + ca) + sa
    x = x + ga * _A_ref(h, A_wq, A_wk, A_wv, A_wo)
    h = _layernorm(x, axis=-1) * (1 + cb) + sb
    x = x + gb * _B_ref(h, B_w_in, B_w_sp, B_b_sp, B_w_out)
    return x
```

```python
import jax
import jax.numpy as jnp
from jax import lax
import jax.experimental.pallas as pl
import jax.experimental.pallas.tpu as pltpu

S = 2048
D = 512
H = 32
DH = 16
F = 1792
FH = F // 2
EPS = 1e-5
LOG2E = 1.4426950408889634
QK_SCALE = (DH ** -0.5) * LOG2E

RB = 256
NRB = S // RB
TQ = 512
TK = 128
LAG = 2
NU = 4

NREP = 6.0
SIG = 40.0
LOGIT_BOUND = 60.0
V_HI = 2.0 ** 40
V_LO = 2.0 ** -40

f32 = jnp.float32
bf16 = jnp.bfloat16


def _nt(a, b):
    return lax.dot_general(a, b, (((1,), (1,)), ((), ())), preferred_element_type=f32)


def _nn(a, b):
    return jnp.dot(a, b, preferred_element_type=f32)


def _ln(x):
    m = jnp.mean(x, axis=-1, keepdims=True)
    xc = x - m
    v = jnp.mean(xc * xc, axis=-1, keepdims=True)
    return xc * lax.rsqrt(v + EPS)


def _gelu_tanh(x):
    c0 = 0.7978845608028654
    c1 = 0.044715 * c0
    u = x * (c0 + c1 * (x * x))
    hx = 0.5 * x
    return hx + hx * jnp.tanh(u)


def _rnd(x):
    magic = 12582912.0
    return (x + magic) - magic


def _to_i8(x):
    return x.astype(jnp.int32).astype(jnp.int8)


def _kernel(x_hbm, wq_hbm, wk_ref, wv_ref, wo_hbm, win_hbm, wsp_hbm, bsp_ref, wout_hbm, c_ref, wmod_hbm,
            out_hbm,
            x_v, wq_v, wo_v, win_v, wsp_v, wout_v, wmod_v,
            mod_v, wt_v, wkrep_v, bcol_v,
            q8_v, qt_v, qsc_v, kf_v, k8_v, vt_v, stat_v, ot_v,
            x1_v, z1_v, z2_v, out_v,
            xsem, wsem, osem):
    def x_copy(i):
        r = pl.ds(pl.multiple_of(i * RB, RB), RB)
        return pltpu.make_async_copy(x_hbm.at[r], x_v.at[r], xsem.at[i])

    def out_copy(i):
        r = pl.ds(pl.multiple_of(i * RB, RB), RB)
        return pltpu.make_async_copy(out_v.at[r], out_hbm.at[r], osem.at[i])

    cp_moda = pltpu.make_async_copy(wmod_hbm.at[:, 0:2 * D], wmod_v.at[:, 0:2 * D], wsem.at[0])
    cp_wq = pltpu.make_async_copy(wq_hbm, wq_v, wsem.at[1])
    cp_modb = pltpu.make_async_copy(wmod_hbm.at[:, 2 * D:6 * D], wmod_v.at[:, 2 * D:6 * D], wsem.at[2])
    cp_wo = pltpu.make_async_copy(wo_hbm, wo_v, wsem.at[3])
    cp_win = pltpu.make_async_copy(win_hbm, win_v, wsem.at[4])
    cp_wsp = pltpu.make_async_copy(wsp_hbm, wsp_v, wsem.at[5])
    cp_wout = pltpu.make_async_copy(wout_hbm, wout_v, wsem.at[6])

    cp_wq.start()
    cp_moda.start()
    for i in range(NRB):
        x_copy(i).start()
    cp_modb.start()
    cp_wo.start()
    cp_win.start()
    cp_wsp.start()
    cp_wout.start()

    eye16 = (lax.broadcasted_iota(jnp.int32, (DH, DH), 0)
             == lax.broadcasted_iota(jnp.int32, (DH, DH), 1)).astype(f32).astype(bf16)
    rep16 = (lax.broadcasted_iota(jnp.int32, (DH, 128), 0)
             == lax.broadcasted_iota(jnp.int32, (DH, 128), 1) % DH).astype(f32).astype(bf16)
    wk = wk_ref[...]
    wv = wv_ref[...]
    wt_v[D:D + DH, :] = _nt(eye16, wv).astype(bf16)
    wt_v[D + DH:D + 2 * DH, :] = _nt(eye16, wk).astype(bf16)
    wkrep_v[...] = _nn(wk, rep16).astype(bf16)
    brow = jnp.broadcast_to(bsp_ref[...].astype(f32), (128, S))
    bcol_v[...] = brow.T

    c = c_ref[...].astype(f32)
    sc = jnp.broadcast_to(c * jax.nn.sigmoid(c), (16, D)).astype(bf16)

    cp_wq.wait()
    wt_v[0:D, :] = wq_v[...].astype(f32).T.astype(bf16)
    cp_moda.wait()
    mod_v[:, 0:2 * D] = _nn(sc, wmod_v[:, 0:2 * D])[0:8]

    stat_v[...] = jnp.zeros(stat_v.shape, f32)

    def phase1(i, carry):
        x_copy(i).wait()
        r0 = pl.multiple_of(i * RB, RB)
        rows = pl.ds(r0, RB)
        x = x_v[rows, :].astype(f32)
        sa = mod_v[0:1, 0:D]
        ca = mod_v[0:1, D:2 * D]
        h = (_ln(x) * (1.0 + ca) + sa).astype(bf16)
        kf_v[rows, :] = _nn(h, wkrep_v[...])
        t = _nt(wt_v[...], h)
        vT = t[D:D + DH]
        kT = t[D + DH:D + 2 * DH]
        vt_v[:, rows] = vT.astype(bf16)
        qT = t[0:D] * QK_SCALE
        qt_v[:, rows] = qT.astype(bf16)
        q3 = qT.reshape(H, DH, RB)
        qmax = jnp.max(jnp.abs(q3), axis=1, keepdims=True)
        qn2 = jnp.sum(q3 * q3, axis=1, keepdims=True)
        qmax = jnp.maximum(qmax, 1e-30)
        qf = q3 * (127.0 / qmax)
        qh = _rnd(qf)
        qr = _rnd((qf - qh) * SIG)
        qc = _rnd(qf * (NREP / SIG))
        q8_v[:, :, rows] = _to_i8(jnp.concatenate([qh, qh, qc, qr], axis=1))
        qsc_v[:, :, rows] = jnp.broadcast_to(qmax * (1.0 / (127.0 * NREP)), (H, 8, RB))
        st = stat_v[...]
        upd = jnp.concatenate([
            jnp.max(qn2, axis=0),
            jnp.sum(kT * kT, axis=0, keepdims=True),
            jnp.max(jnp.abs(kT), axis=0, keepdims=True),
            jnp.max(jnp.abs(vT), axis=0, keepdims=True),
            jnp.zeros((4, RB), f32)], axis=0)
        stat_v[...] = jnp.maximum(st, upd)
        return carry

    lax.fori_loop(0, NRB, phase1, 0)

    st = stat_v[...]
    qn2max = jnp.max(st[0:1])
    kn2max = jnp.max(st[1:2])
    kmax = jnp.max(st[2:3])
    vmax = jnp.max(st[3:4])
    safe = jnp.logical_and(qn2max * kn2max <= LOGIT_BOUND * LOGIT_BOUND,
                           jnp.logical_and(vmax <= V_HI, vmax >= V_LO))

    nq = S // TQ
    nk = S // TK

    @pl.when(safe)
    def _attention_fast():
        kmx = jnp.maximum(jnp.max(st[2:3], axis=1, keepdims=True), 1e-30)
        kf = kf_v[...] * (127.0 / kmx)
        kh = _rnd(kf)
        kr = _rnd((kf - kh) * SIG)
        kc = _rnd(kh * (NREP / SIG))
        lane = lax.broadcasted_iota(jnp.int32, (S, 128), 1)
        k8_v[...] = _to_i8(jnp.where(lane < 96, kh, jnp.where(lane < 112, kr, kc)))
        kinv = kmx * (1.0 / 127.0)

        def body(it, carry):
            units = []
            for u in range(NU):
                iu = it * NU + u
                units.append((iu // nq, pl.multiple_of((iu % nq) * TQ, TQ)))
            chunks = [(u, j) for u in range(NU) for j in range(nk)]
            acc = [jnp.zeros((DH, TQ), f32) for _ in range(NU)]
            den = [jnp.zeros((8, TQ), f32) for _ in range(NU)]
            ps = {}

            def pv(idx):
                u, j = chunks[idx]
                acc[u] = acc[u] + _nn(vt_v[:, j * TK:(j + 1) * TK], ps.pop(idx))
                if j == nk - 1:
                    hh, qs = units[u]
                    l = jnp.sum(den[u], axis=0, keepdims=True)
                    ot_v[pl.ds(pl.multiple_of(hh * DH, DH), DH), pl.ds(qs, TQ)] = acc[u] * (1.0 / l)

            for idx, (u, j) in enumerate(chunks):
                hh, qs = units[u]
                qa = q8_v[hh, 0:32, pl.ds(qs, TQ)]
                qb = q8_v[hh, 32:64, pl.ds(qs, TQ)]
                qw = jnp.concatenate([qa, qa, qa, qb], axis=0)
                scl = qsc_v[hh, :, pl.ds(qs, TQ)] * kinv
                s = jnp.dot(k8_v[j * TK:(j + 1) * TK, :], qw, preferred_element_type=jnp.int32).astype(f32)
                p = jnp.exp2(s.reshape(TK // 8, 8, TQ) * scl[None])
                den[u] = den[u] + jnp.sum(p, axis=0)
                ps[idx] = p.reshape(TK, TQ).astype(bf16)
                if idx >= LAG:
                    pv(idx - LAG)
            for idx in range(len(chunks) - LAG, len(chunks)):
                pv(idx)
            return carry

        lax.fori_loop(0, H * nq // NU, body, 0)

    @pl.when(jnp.logical_not(safe))
    def _attention_exact_max():
        tq = 128

        def body(it, carry):
            hh = it // (S // tq)
            qs = pl.multiple_of((it % (S // tq)) * tq, tq)
            hrows = pl.ds(pl.multiple_of(hh * DH, DH), DH)
            kb = kf_v[...][:, 0:DH].astype(bf16)
            s = _nn(kb, qt_v[hrows, pl.ds(qs, tq)])
            m = jnp.max(s, axis=0, keepdims=True)
            p = jnp.exp2(s - m)
            l = jnp.sum(p, axis=0, keepdims=True)
            o = _nn(vt_v[...], p.astype(bf16))
            ot_v[hrows, pl.ds(qs, tq)] = o / l
            return carry

        lax.fori_loop(0, H * (S // tq), body, 0)

    cp_modb.wait()
    mod_v[:, 2 * D:6 * D] = _nn(sc, wmod_v[:, 2 * D:6 * D])[0:8]
    cp_wo.wait()
    cp_win.wait()

    def phase3(i, carry):
        rows = pl.ds(pl.multiple_of(i * RB, RB), RB)
        o = ot_v[:, rows].T.astype(bf16)
        a = _nn(o, wo_v[...])
        ga = mod_v[0:1, 2 * D:3 * D]
        sb = mod_v[0:1, 3 * D:4 * D]
        cb = mod_v[0:1, 4 * D:5 * D]
        x1 = x_v[rows, :].astype(f32) + ga * a
        x1_v[rows, :] = x1
        h = (_ln(x1) * (1.0 + cb) + sb).astype(bf16)
        z1_v[rows, :] = _gelu_tanh(_nn(h, win_v[:, 0:FH]))
        z2_v[rows, :] = _ln(_gelu_tanh(_nn(h, win_v[:, FH:F]))).astype(bf16)
        return carry

    lax.fori_loop(0, NRB, phase3, 0)

    cp_wsp.wait()
    cp_wout.wait()

    def phase4(i, carry):
        rows = pl.ds(pl.multiple_of(i * RB, RB), RB)
        g = _nn(wsp_v[rows, :], z2_v[...])
        bc = bcol_v[rows, :]
        g = g + jnp.concatenate([bc] * (FH // 128), axis=1)
        u = (z1_v[rows, :] * g).astype(bf16)
        y = _nn(u, wout_v[...])
        gb = mod_v[0:1, 5 * D:6 * D]
        out_v[rows, :] = (x1_v[rows, :] + gb * y).astype(bf16)
        out_copy(i).start()
        return carry

    lax.fori_loop(0, NRB, phase4, 0)
    for i in range(NRB):
        out_copy(i).wait()


@jax.jit
def pallas_adaLN_cond__grouped_kv_mqa__mixer_gmlp__prompt_kernel(
    A_x: jax.Array,
    A_wq: jax.Array,
    A_wk: jax.Array,
    A_wv: jax.Array,
    A_wo: jax.Array,
    B_x: jax.Array,
    B_w_in: jax.Array,
    B_w_sp: jax.Array,
    B_b_sp: jax.Array,
    B_w_out: jax.Array,
    c: jax.Array,
    w_mod: jax.Array,
):
    del B_x
    hbm = pl.BlockSpec(memory_space=pl.ANY)
    vmem = pl.BlockSpec(memory_space=pltpu.VMEM)
    scratch = [
        pltpu.VMEM((S, D), bf16),
        pltpu.VMEM((D, D), bf16),
        pltpu.VMEM((D, D), bf16),
        pltpu.VMEM((D, F), bf16),
        pltpu.VMEM((S, S), bf16),
        pltpu.VMEM((FH, D), bf16),
        pltpu.VMEM((D, 6 * D), bf16),
        pltpu.VMEM((8, 6 * D), f32),
        pltpu.VMEM((D + 2 * DH, D), bf16),
        pltpu.VMEM((D, 128), bf16),
        pltpu.VMEM((S, 128), f32),
        pltpu.VMEM((H, 64, S), jnp.int8),
        pltpu.VMEM((D, S), bf16),
        pltpu.VMEM((H, 8, S), f32),
        pltpu.VMEM((S, 128), f32),
        pltpu.VMEM((S, 128), jnp.int8),
        pltpu.VMEM((DH, S), bf16),
        pltpu.VMEM((8, RB), f32),
        pltpu.VMEM((D, S), f32),
        pltpu.VMEM((S, D), f32),
        pltpu.VMEM((S, FH), f32),
        pltpu.VMEM((S, FH), bf16),
        pltpu.VMEM((S, D), bf16),
        pltpu.SemaphoreType.DMA((NRB,)),
        pltpu.SemaphoreType.DMA((7,)),
        pltpu.SemaphoreType.DMA((NRB,)),
    ]
    out = pl.pallas_call(
        _kernel,
        out_shape=jax.ShapeDtypeStruct((S, D), bf16),
        in_specs=[hbm, hbm, vmem, vmem, hbm, hbm, hbm, vmem, hbm, vmem, hbm],
        out_specs=hbm,
        scratch_shapes=scratch,
        compiler_params=pltpu.CompilerParams(vmem_limit_bytes=100 * 1024 * 1024),
    )(A_x.reshape(S, D), A_wq, A_wk, A_wv, A_wo, B_w_in, B_w_sp, B_b_sp.reshape(1, S), B_w_out, c, w_mod)
    return out.reshape(1, S, D)
```

```python
import jax
import jax.numpy as jnp
from jax import lax
import jax.experimental.pallas as pl
import jax.experimental.pallas.tpu as pltpu

S = 2048
D = 512
H = 32
DH = 16
F = 1792
FH = F // 2
EPS = 1e-5
LOG2E = 1.4426950408889634
QK_SCALE = (DH ** -0.5) * LOG2E

RB = 256
NRB = S // RB
P3 = 2
TQ = 512
TK = 256
LAG = 1
NU = 8

NREP = 6.0
SIG = 40.0
LOGIT_BOUND = 60.0
V_HI = 2.0 ** 40
V_LO = 2.0 ** -40

f32 = jnp.float32
bf16 = jnp.bfloat16


def _nt(a, b):
    return lax.dot_general(a, b, (((1,), (1,)), ((), ())), preferred_element_type=f32)


def _nn(a, b):
    return jnp.dot(a, b, preferred_element_type=f32)


def _ln(x):
    m = jnp.mean(x, axis=-1, keepdims=True)
    xc = x - m
    v = jnp.mean(xc * xc, axis=-1, keepdims=True)
    return xc * lax.rsqrt(v + EPS)


def _gelu_tanh(x):
    c0 = 0.7978845608028654
    c1 = 0.044715 * c0
    u = x * (c0 + c1 * (x * x))
    hx = 0.5 * x
    return hx + hx * jnp.tanh(u)


MAGIC = 12582912.0


def _low_byte(t):
    return pltpu.bitcast(t, jnp.int32).astype(jnp.int8)


def _recip(x):
    r = pl.reciprocal(x, approx=True)
    return r * (2.0 - x * r)


def _kernel(x_hbm, wq_hbm, wkt_ref, wvt_ref, wo_hbm, win_hbm, wsp_hbm, bsp_ref, wout_hbm, c_ref, wmod_hbm,
            out_hbm,
            x_v, wq_v, wo_v, win_v, wsp_v, wout_v, wmod_v,
            mod_v, mod_b, wt_v,
            q8_v, qsc_v, kt_v, kb_v, k8_v, vt_v, ot_v,
            x1_v, z1_v, z2_v, out_v,
            xsem, wsem, osem):
    def x_copy(i):
        r = pl.ds(i * RB, RB)
        return pltpu.make_async_copy(x_hbm.at[r], x_v.at[r], xsem.at[i])

    def out_copy(i):
        r = pl.ds(pl.multiple_of(i * RB, RB), RB)
        return pltpu.make_async_copy(out_v.at[r], out_hbm.at[r], osem.at[i])

    cp_moda = pltpu.make_async_copy(wmod_hbm.at[:, 0:2 * D], wmod_v.at[:, 0:2 * D], wsem.at[0])
    cp_wq = pltpu.make_async_copy(wq_hbm, wq_v, wsem.at[1])
    cp_modb = pltpu.make_async_copy(wmod_hbm.at[:, 2 * D:6 * D], wmod_v.at[:, 2 * D:6 * D], wsem.at[2])
    cp_wo = pltpu.make_async_copy(wo_hbm, wo_v, wsem.at[3])
    cp_win = pltpu.make_async_copy(win_hbm, win_v, wsem.at[4])
    cp_wsp = pltpu.make_async_copy(wsp_hbm, wsp_v, wsem.at[5])
    cp_wout = pltpu.make_async_copy(wout_hbm, wout_v, wsem.at[6])

    cp_wq.start()
    cp_moda.start()
    for i in range(NRB):
        x_copy(i).start()

    wt_v[D:D + DH, :] = wvt_ref[...]
    wt_v[D + DH:D + 2 * DH, :] = wkt_ref[...]
    mod_b[...] = bsp_ref[...].astype(f32)
    c = c_ref[...].astype(f32)
    sc = jnp.broadcast_to(c * jax.nn.sigmoid(c), (16, D)).astype(bf16)

    cp_wq.wait()
    wt_v[0:D, :] = wq_v[...].astype(f32).T.astype(bf16)
    cp_moda.wait()
    moda = _nn(sc, wmod_v[:, 0:2 * D])
    sa = moda[0:1, 0:D]
    ca1 = 1.0 + moda[0:1, D:2 * D]

    def ln1(i):
        x_copy(i).wait()
        x = x_v[i * RB:(i + 1) * RB, :].astype(f32)
        return (_ln(x) * ca1 + sa).astype(bf16)

    def proj(i, h):
        cols = slice(i * RB, (i + 1) * RB)
        t = _nt(wt_v[...], h)
        vT = t[D:D + DH]
        vt_v[:, cols] = vT.astype(bf16)
        kt_v[:, cols] = t[D + DH:D + 2 * DH]
        qT = t[0:D]
        ot_v[:, cols] = qT
        q3 = qT.reshape(H, DH, RB)
        qmax = jnp.maximum(jnp.max(jnp.abs(q3), axis=1, keepdims=True), 1e-30)
        qn2 = jnp.sum(q3 * q3, axis=1, keepdims=True)
        qf = q3 * (127.0 * _recip(qmax))
        th = qf + MAGIC
        tr = (qf - (th - MAGIC)) * SIG + MAGIC
        tc = qf * (NREP / SIG) + MAGIC
        q8_v[:, :, cols] = _low_byte(jnp.concatenate([th, th, tc, tr], axis=1))
        qsc_v[:, :, cols] = jnp.broadcast_to(qmax, (H, 8, RB))
        return jnp.max(qn2, axis=0), jnp.max(jnp.abs(vT), axis=0, keepdims=True)

    h = ln1(0)
    qn2max = vmax = None
    for i in range(NRB):
        hn = ln1(i + 1) if i + 1 < NRB else None
        a, b = proj(i, h)
        qn2max = a if qn2max is None else jnp.maximum(qn2max, a)
        vmax = b if vmax is None else jnp.maximum(vmax, b)
        h = hn

    cp_modb.start()
    cp_wo.start()
    cp_win.start()
    cp_wsp.start()
    cp_wout.start()

    kT = kt_v[...]
    kn2max = jnp.max(jnp.sum(kT * kT, axis=0, keepdims=True))
    vmx = jnp.max(vmax)
    safe = jnp.logical_and(jnp.max(qn2max) * kn2max <= (LOGIT_BOUND / QK_SCALE) ** 2,
                           jnp.logical_and(vmx <= V_HI, vmx >= V_LO))

    nq = S // TQ
    nk = S // TK

    @pl.when(safe)
    def _attention_fast():
        kmx = jnp.max(jnp.max(jnp.abs(kT), axis=0, keepdims=True), axis=1, keepdims=True)
        kmx = jnp.maximum(kmx, 1e-30)
        kf = kT * (127.0 / kmx)
        th = kf + MAGIC
        kh = th - MAGIC
        tr = (kf - kh) * SIG + MAGIC
        tc = kh * (NREP / SIG) + MAGIC
        k8_v[...] = _low_byte(jnp.concatenate([th] * 6 + [tr, tc], axis=0).T)
        kscale = kmx * (QK_SCALE / (127.0 * 127.0 * NREP))

        def body(it, carry):
            units = []
            for u in range(NU):
                iu = it * NU + u
                units.append((iu // nq, pl.multiple_of((iu % nq) * TQ, TQ)))
            chunks = [(u, j) for u in range(NU) for j in range(nk)]
            acc = [None] * NU
            den = [None] * NU
            ps = {}

            def pv(idx):
                u, j = chunks[idx]
                o = _nn(vt_v[:, j * TK:(j + 1) * TK], ps.pop(idx))
                acc[u] = o if j == 0 else o + acc[u]
                if j == nk - 1:
                    hh, qs = units[u]
                    l = jnp.sum(den[u], axis=0, keepdims=True)
                    ot_v[pl.ds(pl.multiple_of(hh * DH, DH), DH), pl.ds(qs, TQ)] = acc[u] * (1.0 / l)

            for idx, (u, j) in enumerate(chunks):
                hh, qs = units[u]
                qa = q8_v[hh, 0:32, pl.ds(qs, TQ)]
                qb = q8_v[hh, 32:64, pl.ds(qs, TQ)]
                qw = jnp.concatenate([qa, qa, qa, qb], axis=0)
                scl = qsc_v[hh, :, pl.ds(qs, TQ)] * kscale
                s = jnp.dot(k8_v[j * TK:(j + 1) * TK, :], qw, preferred_element_type=jnp.int32).astype(f32)
                p = jnp.exp2(s.reshape(TK // 8, 8, TQ) * scl[None])
                d = jnp.sum(p, axis=0)
                den[u] = d if j == 0 else den[u] + d
                ps[idx] = p.reshape(TK, TQ).astype(bf16)
                if idx >= LAG:
                    pv(idx - LAG)
            for idx in range(len(chunks) - LAG, len(chunks)):
                pv(idx)
            return carry

        lax.fori_loop(0, H * nq // NU, body, 0)

    @pl.when(jnp.logical_not(safe))
    def _attention_exact_max():
        tq = 128
        kb_v[...] = jnp.concatenate([kT] * 8, axis=0).T.astype(bf16)

        def body(it, carry):
            hh = it // (S // tq)
            qs = pl.multiple_of((it % (S // tq)) * tq, tq)
            hrows = pl.ds(pl.multiple_of(hh * DH, DH), DH)
            q = ot_v[hrows, pl.ds(qs, tq)].astype(bf16)
            s = _nn(kb_v[...][:, 0:DH], q) * QK_SCALE
            m = jnp.max(s, axis=0, keepdims=True)
            p = jnp.exp2(s - m)
            l = jnp.sum(p, axis=0, keepdims=True)
            o = _nn(vt_v[...], p.astype(bf16))
            ot_v[hrows, pl.ds(qs, tq)] = o / l
            return carry

        lax.fori_loop(0, H * (S // tq), body, 0)

    cp_modb.wait()
    mod_v[...] = _nn(sc, wmod_v[:, 2 * D:6 * D])[0:8]
    cp_wo.wait()
    cp_win.wait()

    def phase3(i, carry):
        ga = mod_v[0:1, 0:D]
        sb = mod_v[0:1, D:2 * D]
        cb1 = 1.0 + mod_v[0:1, 2 * D:3 * D]
        rows = [pl.ds(pl.multiple_of((i * P3 + k) * RB, RB), RB) for k in range(P3)]
        hs = []
        for r in rows:
            o = ot_v[:, r].T.astype(bf16)
            x1 = x_v[r, :].astype(f32) + ga * _nn(o, wo_v[...])
            x1_v[r, :] = x1
            hs.append((_ln(x1) * cb1 + sb).astype(bf16))
        for r, h2 in zip(rows, hs):
            z2_v[r, :] = _ln(_gelu_tanh(_nn(h2, win_v[:, FH:F]))).astype(bf16)
            z1_v[r, :] = _gelu_tanh(_nn(h2, win_v[:, 0:FH]))
        return carry

    lax.fori_loop(0, NRB // P3, phase3, 0)

    cp_wsp.wait()
    cp_wout.wait()

    def phase4(i, carry):
        rows = pl.ds(pl.multiple_of(i * RB, RB), RB)
        g = _nn(wsp_v[rows, :], z2_v[...])
        bc = jnp.concatenate(
            [jnp.broadcast_to(mod_b[pl.ds(i * (RB // 128) + k, 1), :], (128, 128)).T for k in range(RB // 128)],
            axis=0)
        g = g + jnp.concatenate([bc] * (FH // 128), axis=1)
        u = (z1_v[rows, :] * g).astype(bf16)
        y = _nn(u, wout_v[...])
        gb = mod_v[0:1, 3 * D:4 * D]
        out_v[rows, :] = (x1_v[rows, :] + gb * y).astype(bf16)
        out_copy(i).start()
        return carry

    lax.fori_loop(0, NRB, phase4, 0)
    for i in range(NRB):
        out_copy(i).wait()


@jax.jit
def pallas_adaLN_cond__grouped_kv_mqa__mixer_gmlp__prompt_kernel(
    A_x: jax.Array,
    A_wq: jax.Array,
    A_wk: jax.Array,
    A_wv: jax.Array,
    A_wo: jax.Array,
    B_x: jax.Array,
    B_w_in: jax.Array,
    B_w_sp: jax.Array,
    B_b_sp: jax.Array,
    B_w_out: jax.Array,
    c: jax.Array,
    w_mod: jax.Array,
):
    del B_x
    hbm = pl.BlockSpec(memory_space=pl.ANY)
    vmem = pl.BlockSpec(memory_space=pltpu.VMEM)
    scratch = [
        pltpu.VMEM((S, D), bf16),
        pltpu.VMEM((D, D), bf16),
        pltpu.VMEM((D, D), bf16),
        pltpu.VMEM((D, F), bf16),
        pltpu.VMEM((S, S), bf16),
        pltpu.VMEM((FH, D), bf16),
        pltpu.VMEM((D, 6 * D), bf16),
        pltpu.VMEM((8, 4 * D), f32),
        pltpu.VMEM((S // 128, 128), f32),
        pltpu.VMEM((D + 2 * DH, D), bf16),
        pltpu.VMEM((H, 64, S), jnp.int8),
        pltpu.VMEM((H, 8, S), f32),
        pltpu.VMEM((DH, S), f32),
        pltpu.VMEM((S, 128), bf16),
        pltpu.VMEM((S, 128), jnp.int8),
        pltpu.VMEM((DH, S), bf16),
        pltpu.VMEM((D, S), f32),
        pltpu.VMEM((S, D), f32),
        pltpu.VMEM((S, FH), f32),
        pltpu.VMEM((S, FH), bf16),
        pltpu.VMEM((S, D), bf16),
        pltpu.SemaphoreType.DMA((NRB,)),
        pltpu.SemaphoreType.DMA((7,)),
        pltpu.SemaphoreType.DMA((NRB,)),
    ]
    out = pl.pallas_call(
        _kernel,
        out_shape=jax.ShapeDtypeStruct((S, D), bf16),
        in_specs=[hbm, hbm, vmem, vmem, hbm, hbm, hbm, vmem, hbm, vmem, hbm],
        out_specs=hbm,
        scratch_shapes=scratch,
        compiler_params=pltpu.CompilerParams(vmem_limit_bytes=100 * 1024 * 1024),
    )(A_x.reshape(S, D), A_wq, A_wk.T, A_wv.T, A_wo, B_w_in, B_w_sp, B_b_sp.reshape(S // 128, 128), B_w_out, c, w_mod)
    return out.reshape(1, S, D)
```

```python
import jax
import jax.numpy as jnp
from jax import lax
import jax.experimental.pallas as pl
import jax.experimental.pallas.tpu as pltpu

S = 2048
D = 512
H = 32
DH = 16
F = 1792
FH = F // 2
EPS = 1e-5
LOG2E = 1.4426950408889634
QK_SCALE = (DH ** -0.5) * LOG2E

RB = 256
NRB = S // RB
P3 = 2
TQ = 512
TK = 256
LAG = 1
NU = 8
NQ = S // TQ
NBODY = H * NQ // NU

NREP = 6.0
SIG = 40.0
LOGIT_BOUND = 60.0
V_HI = 2.0 ** 40
V_LO = 2.0 ** -40

f32 = jnp.float32
bf16 = jnp.bfloat16


def _nt(a, b):
    return lax.dot_general(a, b, (((1,), (1,)), ((), ())), preferred_element_type=f32)


def _nn(a, b):
    return jnp.dot(a, b, preferred_element_type=f32)


def _ln(x):
    m = jnp.mean(x, axis=-1, keepdims=True)
    xc = x - m
    v = jnp.mean(xc * xc, axis=-1, keepdims=True)
    return xc * lax.rsqrt(v + EPS)


def _gelu_tanh(x):
    c0 = 0.7978845608028654
    c1 = 0.044715 * c0
    u = x * (c0 + c1 * (x * x))
    hx = 0.5 * x
    return hx + hx * jnp.tanh(u)


MAGIC = 12582912.0


def _low_byte(t):
    return pltpu.bitcast(t, jnp.int32).astype(jnp.int8)


def _recip(x):
    r = pl.reciprocal(x, approx=True)
    return r * (2.0 - x * r)


def _quant_q(q3, eps=1e-30):
    qmax = jnp.maximum(jnp.max(jnp.abs(q3), axis=-2, keepdims=True), eps)
    qf = q3 * (127.0 * _recip(qmax))
    th = qf + MAGIC
    tr = (qf - (th - MAGIC)) * SIG + MAGIC
    tc = qf * (NREP / SIG) + MAGIC
    return _low_byte(jnp.concatenate([th, th, tc, tr], axis=-2)), qmax


XG = [(0, 1), (1, 3), (3, 5), (5, 8)]


def _kernel(x_hbm, wq_hbm, wkt_hbm, wvt_hbm, wo_hbm, win_hbm, wsp_hbm, bsp_hbm, wout_hbm, c_hbm, wmod_hbm,
            out_hbm,
            x_v, wq_v, wo_v, win_v, wsp_v, wout_v, wmod_v, c_v, bsp_v,
            mod_v, mod_b, wt_v,
            q8_v, qsc_v, kt_v, kb_v, k8_v, ksc_v, vt_v, qt_v, ot_v,
            x1_v, z1_v, z2_v, out_v,
            xsem, wsem, osem):
    def x_copy(g):
        r = pl.ds(XG[g][0] * RB, (XG[g][1] - XG[g][0]) * RB)
        return pltpu.make_async_copy(x_hbm.at[r], x_v.at[r], xsem.at[g])

    def out_copy(i):
        r = pl.ds(pl.multiple_of(i * RB, RB), RB)
        return pltpu.make_async_copy(out_v.at[r], out_hbm.at[r], osem.at[i])

    cp_moda = pltpu.make_async_copy(wmod_hbm.at[:, 0:2 * D], wmod_v.at[:, 0:2 * D], wsem.at[0])
    cp_wq = pltpu.make_async_copy(wq_hbm, wq_v, wsem.at[1])
    cp_modb = pltpu.make_async_copy(wmod_hbm.at[:, 2 * D:6 * D], wmod_v.at[:, 2 * D:6 * D], wsem.at[2])
    cp_wo = pltpu.make_async_copy(wo_hbm, wo_v, wsem.at[3])
    cp_win = pltpu.make_async_copy(win_hbm, win_v, wsem.at[4])
    cp_wsp = pltpu.make_async_copy(wsp_hbm, wsp_v, wsem.at[5])
    cp_wout = pltpu.make_async_copy(wout_hbm, wout_v, wsem.at[6])
    cp_c = pltpu.make_async_copy(c_hbm, c_v, wsem.at[7])
    cp_wk = pltpu.make_async_copy(wkt_hbm, wt_v.at[0:DH], wsem.at[8])
    cp_wv = pltpu.make_async_copy(wvt_hbm, wt_v.at[DH:2 * DH], wsem.at[9])
    cp_bsp = pltpu.make_async_copy(bsp_hbm, bsp_v, wsem.at[10])

    x_copy(0).start()
    cp_wq.start()
    cp_moda.start()
    cp_c.start()
    cp_wk.start()
    cp_wv.start()

    def norm1(i):
        return _ln(x_v[i * RB:(i + 1) * RB, :].astype(f32))

    x_copy(0).wait()
    x_copy(1).start()
    n0 = norm1(0)
    cp_wq.wait()
    x_copy(2).start()
    wt_v[2 * DH:2 * DH + D, :] = wq_v[...].astype(f32).T.astype(bf16)
    cp_c.wait()
    cp_wk.wait()
    cp_wv.wait()
    cp_moda.wait()
    x_copy(3).start()
    x_copy(1).wait()
    c = c_v[...].astype(f32)
    sc = jnp.broadcast_to(c * jax.nn.sigmoid(c), (16, D)).astype(bf16)
    moda = _nn(sc, wmod_v[:, 0:2 * D])
    sa = moda[0:1, 0:D]
    ca1 = 1.0 + moda[0:1, D:2 * D]

    def proj(i, h):
        cols = slice(i * RB, (i + 1) * RB)
        t = _nt(wt_v[...], h)
        kT = t[0:DH]
        kt_v[:, cols] = kT
        kmx = jnp.max(jnp.max(jnp.abs(kT), axis=0, keepdims=True), axis=1, keepdims=True)
        kmx = jnp.maximum(kmx, 1e-30)
        kf = kT * (127.0 * _recip(kmx))
        th = kf + MAGIC
        kh = th - MAGIC
        tr = (kf - kh) * SIG + MAGIC
        tc = kh * (NREP / SIG) + MAGIC
        k8_v[cols, :] = _low_byte(jnp.concatenate([th] * 6 + [tr, tc], axis=0).T)
        ksc_v[i] = jnp.broadcast_to(kmx * (QK_SCALE / (127.0 * 127.0 * NREP)), (8, 128))
        vT = t[DH:2 * DH]
        vt_v[:, cols] = vT
        qT = t[2 * DH:2 * DH + D]
        qt_v[:, cols] = qT
        q3 = qT.reshape(H, DH, RB)
        q8, qmax = _quant_q(q3[0:NU // NQ])
        qc = slice((i * RB) % TQ, (i * RB) % TQ + RB)
        for hh in range(NU // NQ):
            u = hh * NQ + (i * RB) // TQ
            q8_v[u, :, qc] = q8[hh]
            qsc_v[u, :, qc] = jnp.broadcast_to(qmax[hh], (8, RB))
        q2 = q3 * q3
        qb = jnp.max(q2[:, 0:8] + q2[:, 8:16], axis=0)
        return qb, jnp.sum(kT * kT, axis=0, keepdims=True), jnp.max(jnp.abs(vT), axis=0, keepdims=True)

    h = (n0 * ca1 + sa).astype(bf16)
    stats = None
    for i in range(NRB):
        for g in range(2, len(XG)):
            if XG[g][0] == i + 1:
                x_copy(g).wait()
        hn = (norm1(i + 1) * ca1 + sa).astype(bf16) if i + 1 < NRB else None
        st = proj(i, h)
        stats = st if stats is None else tuple(jnp.maximum(a, b) for a, b in zip(stats, st))
        h = hn

    cp_modb.start()
    cp_wo.start()
    cp_win.start()
    cp_wsp.start()
    cp_wout.start()
    cp_bsp.start()

    qn2max = jnp.max(jnp.sum(stats[0], axis=0, keepdims=True))
    kn2max = jnp.max(stats[1])
    vmx = jnp.max(stats[2])
    safe = jnp.logical_and(qn2max * kn2max <= (LOGIT_BOUND / QK_SCALE) ** 2,
                           jnp.logical_and(vmx <= V_HI, vmx >= V_LO))

    nq = S // TQ
    nk = S // TK

    @pl.when(safe)
    def _attention_fast():
        def body(it, carry):
            chunks = [(u, j) for u in range(NU) for j in range(nk)]
            acc = [None] * NU
            den = [None] * NU
            ps = {}
            itn = jnp.minimum(it + 1, NBODY - 1)

            def rows(i, u):
                return pl.ds(pl.multiple_of((i * (NU // NQ) + u // NQ) * DH, DH), DH)

            def cols(u):
                return slice((u % NQ) * TQ, (u % NQ + 1) * TQ)

            def pv(idx):
                u, j = chunks[idx]
                o = _nn(vt_v[:, j * TK:(j + 1) * TK], ps.pop(idx))
                acc[u] = o if j == 0 else o + acc[u]
                if j == nk - 1:
                    l = jnp.sum(den[u], axis=0, keepdims=True)
                    ot_v[rows(it, u), cols(u)] = acc[u] * (1.0 / l)

            for idx, (u, j) in enumerate(chunks):
                qa = q8_v[u, 0:32, :]
                qb = q8_v[u, 32:64, :]
                qw = jnp.concatenate([qa, qa, qa, qb], axis=0)
                scl = qsc_v[u] * jnp.concatenate([ksc_v[j]] * (TQ // 128), axis=1)
                s = jnp.dot(k8_v[j * TK:(j + 1) * TK, :], qw, preferred_element_type=jnp.int32).astype(f32)
                p = jnp.exp2(s.reshape(TK // 8, 8, TQ) * scl[None])
                d = jnp.sum(p, axis=0)
                den[u] = d if j == 0 else den[u] + d
                ps[idx] = p.reshape(TK, TQ)
                if j % 2 == 0:
                    un = (u - 1) % NU
                    t = j // 2
                    lc = slice(t * 128, (t + 1) * 128)
                    c0 = (un % NQ) * TQ
                    qn = qt_v[rows(it if u == 0 else itn, un), c0 + t * 128:c0 + (t + 1) * 128]
                    q8, qmax = _quant_q(qn, jnp.minimum(d[0:1, lc], 1e-30))
                    q8_v[un, :, lc] = q8
                    qsc_v[un, :, lc] = jnp.broadcast_to(qmax, (8, 128))
                if idx >= LAG:
                    pv(idx - LAG)
            for idx in range(len(chunks) - LAG, len(chunks)):
                pv(idx)
            return carry

        lax.fori_loop(0, NBODY, body, 0)

    @pl.when(jnp.logical_not(safe))
    def _attention_exact_max():
        tq = 128
        kb_v[...] = jnp.concatenate([kt_v[...]] * 8, axis=0).T.astype(bf16)

        def body(it, carry):
            hh = it // (S // tq)
            qs = pl.multiple_of((it % (S // tq)) * tq, tq)
            hrows = pl.ds(pl.multiple_of(hh * DH, DH), DH)
            q = qt_v[hrows, pl.ds(qs, tq)].astype(bf16)
            s = _nn(kb_v[...][:, 0:DH], q) * QK_SCALE
            m = jnp.max(s, axis=0, keepdims=True)
            p = jnp.exp2(s - m)
            l = jnp.sum(p, axis=0, keepdims=True)
            o = _nn(vt_v[...], p)
            ot_v[hrows, pl.ds(qs, tq)] = o / l
            return carry

        lax.fori_loop(0, H * (S // tq), body, 0)

    cp_modb.wait()
    mod_v[...] = _nn(sc, wmod_v[:, 2 * D:6 * D])[0:8]
    cp_wo.wait()
    cp_win.wait()

    def phase3(i, carry):
        ga = mod_v[0:1, 0:D]
        sb = mod_v[0:1, D:2 * D]
        cb1 = 1.0 + mod_v[0:1, 2 * D:3 * D]
        rows = [pl.ds(pl.multiple_of((i * P3 + k) * RB, RB), RB) for k in range(P3)]
        hs = []
        for r in rows:
            o = ot_v[:, r].T.astype(bf16)
            x1 = x_v[r, :].astype(f32) + ga * _nn(o, wo_v[...])
            x1_v[r, :] = x1
            hs.append((_ln(x1) * cb1 + sb).astype(bf16))
        for r, h2 in zip(rows, hs):
            z2_v[r, :] = _ln(_gelu_tanh(_nn(h2, win_v[:, FH:F]))).astype(bf16)
            z1_v[r, :] = _gelu_tanh(_nn(h2, win_v[:, 0:FH]))
        return carry

    lax.fori_loop(0, NRB // P3, phase3, 0)

    cp_wsp.wait()
    cp_wout.wait()
    cp_bsp.wait()
    mod_b[...] = bsp_v[...].astype(f32)

    def phase4(i, carry):
        rows = pl.ds(pl.multiple_of(i * RB, RB), RB)
        g = _nn(wsp_v[rows, :], z2_v[...])
        bc = jnp.concatenate(
            [jnp.broadcast_to(mod_b[pl.ds(i * (RB // 128) + k, 1), :], (128, 128)).T for k in range(RB // 128)],
            axis=0)
        g = g + jnp.concatenate([bc] * (FH // 128), axis=1)
        u = (z1_v[rows, :] * g).astype(bf16)
        y = _nn(u, wout_v[...])
        gb = mod_v[0:1, 3 * D:4 * D]
        out_v[rows, :] = (x1_v[rows, :] + gb * y).astype(bf16)
        out_copy(i).start()
        return carry

    lax.fori_loop(0, NRB, phase4, 0)
    for i in range(NRB):
        out_copy(i).wait()


@jax.jit
def pallas_adaLN_cond__grouped_kv_mqa__mixer_gmlp__prompt_kernel(
    A_x: jax.Array,
    A_wq: jax.Array,
    A_wk: jax.Array,
    A_wv: jax.Array,
    A_wo: jax.Array,
    B_x: jax.Array,
    B_w_in: jax.Array,
    B_w_sp: jax.Array,
    B_b_sp: jax.Array,
    B_w_out: jax.Array,
    c: jax.Array,
    w_mod: jax.Array,
):
    del B_x
    hbm = pl.BlockSpec(memory_space=pl.ANY)
    scratch = [
        pltpu.VMEM((S, D), bf16),
        pltpu.VMEM((D, D), bf16),
        pltpu.VMEM((D, D), bf16),
        pltpu.VMEM((D, F), bf16),
        pltpu.VMEM((S, S), bf16),
        pltpu.VMEM((FH, D), bf16),
        pltpu.VMEM((D, 6 * D), bf16),
        pltpu.VMEM((1, D), bf16),
        pltpu.VMEM((S // 128, 128), bf16),
        pltpu.VMEM((8, 4 * D), f32),
        pltpu.VMEM((S // 128, 128), f32),
        pltpu.VMEM((D + 2 * DH, D), bf16),
        pltpu.VMEM((NU, 64, TQ), jnp.int8),
        pltpu.VMEM((NU, 8, TQ), f32),
        pltpu.VMEM((DH, S), f32),
        pltpu.VMEM((S, 128), bf16),
        pltpu.VMEM((S, 128), jnp.int8),
        pltpu.VMEM((NRB, 8, 128), f32),
        pltpu.VMEM((DH, S), f32),
        pltpu.VMEM((D, S), f32),
        pltpu.VMEM((D, S), f32),
        pltpu.VMEM((S, D), f32),
        pltpu.VMEM((S, FH), f32),
        pltpu.VMEM((S, FH), bf16),
        pltpu.VMEM((S, D), bf16),
        pltpu.SemaphoreType.DMA((len(XG),)),
        pltpu.SemaphoreType.DMA((11,)),
        pltpu.SemaphoreType.DMA((NRB,)),
    ]
    out = pl.pallas_call(
        _kernel,
        out_shape=jax.ShapeDtypeStruct((S, D), bf16),
        in_specs=[hbm] * 11,
        out_specs=hbm,
        scratch_shapes=scratch,
        compiler_params=pltpu.CompilerParams(vmem_limit_bytes=100 * 1024 * 1024),
    )(A_x.reshape(S, D), A_wq, A_wk.T, A_wv.T, A_wo, B_w_in, B_w_sp, B_b_sp.reshape(S // 128, 128), B_w_out, c, w_mod)
    return out.reshape(1, S, D)
```

```python
import jax
import jax.numpy as jnp
from jax import lax
import jax.experimental.pallas as pl
import jax.experimental.pallas.tpu as pltpu

S = 2048
D = 512
H = 32
DH = 16
F = 1792
FH = F // 2
EPS = 1e-5
LOG2E = 1.4426950408889634
QK_SCALE = (DH ** -0.5) * LOG2E

RB = 256
NRB = S // RB
P3 = 2
TQ = 512
TK = 256
LAG = 1
NU = 16
NQ = S // TQ
NBODY = H * NQ // NU
NSLOT = 4
AHEAD = 2

NREP = 6.0
SIG = 40.0
LOGIT_BOUND = 60.0
V_HI = 2.0 ** 40
V_LO = 2.0 ** -40

f32 = jnp.float32
bf16 = jnp.bfloat16


def _nt(a, b):
    return lax.dot_general(a, b, (((1,), (1,)), ((), ())), preferred_element_type=f32)


def _nn(a, b):
    return jnp.dot(a, b, preferred_element_type=f32)


def _ln(x):
    m = jnp.mean(x, axis=-1, keepdims=True)
    xc = x - m
    v = jnp.mean(xc * xc, axis=-1, keepdims=True)
    return xc * lax.rsqrt(v + EPS)


def _gelu_tanh(x):
    c0 = 0.7978845608028654
    c1 = 0.044715 * c0
    u = x * (c0 + c1 * (x * x))
    hx = 0.5 * x
    return hx + hx * jnp.tanh(u)


MAGIC = 12582912.0


def _low_byte(t):
    return pltpu.bitcast(t, jnp.int32).astype(jnp.int8)


def _recip(x):
    r = pl.reciprocal(x, approx=True)
    return r * (2.0 - x * r)


def _quant_q(q3, eps=1e-30):
    qmax = jnp.maximum(jnp.max(jnp.abs(q3), axis=-2, keepdims=True), eps)
    qf = q3 * (127.0 * _recip(qmax))
    th = qf + MAGIC
    tr = (qf - (th - MAGIC)) * SIG + MAGIC
    tc = qf * (NREP / SIG) + MAGIC
    return _low_byte(jnp.concatenate([th, th, tc, tr], axis=-2)), qmax


XG = [(0, 1), (1, 2), (2, 4), (4, 8)]


def _kernel(x_hbm, wq_hbm, wkt_hbm, wvt_hbm, wo_hbm, win_hbm, wsp_hbm, bsp_hbm, wout_hbm, c_hbm, wmod_hbm,
            out_hbm,
            x_v, wq_v, wo_v, win_v, wsp_v, wout_v, wmod_v, c_v, bsp_v,
            mod_v, mod_b, wt_v,
            q8_v, qsc_v, kt_v, kb_v, k8_v, ksc_v, vt_v, qt_v, ot_v,
            x1_v, z1_v, z2_v, out_v,
            xsem, wsem, osem):
    def x_copy(g):
        r = pl.ds(XG[g][0] * RB, (XG[g][1] - XG[g][0]) * RB)
        return pltpu.make_async_copy(x_hbm.at[r], x_v.at[r], xsem.at[g])

    def out_copy(i):
        r = pl.ds(pl.multiple_of(i * RB, RB), RB)
        return pltpu.make_async_copy(out_v.at[r], out_hbm.at[r], osem.at[i])

    cp_sa = pltpu.make_async_copy(wmod_hbm.at[:, 0:D], wmod_v.at[:, 0:D], wsem.at[0])
    cp_ca = pltpu.make_async_copy(wmod_hbm.at[:, D:2 * D], wmod_v.at[:, D:2 * D], wsem.at[11])
    cp_wq = [pltpu.make_async_copy(wq_hbm.at[:, k * (D // 2):(k + 1) * (D // 2)],
                                   wq_v.at[:, k * (D // 2):(k + 1) * (D // 2)], wsem.at[(1, 12)[k]]) for k in range(2)]
    cp_modb = pltpu.make_async_copy(wmod_hbm.at[:, 2 * D:6 * D], wmod_v.at[:, 2 * D:6 * D], wsem.at[2])
    cp_wo = pltpu.make_async_copy(wo_hbm, wo_v, wsem.at[3])
    cp_win = pltpu.make_async_copy(win_hbm, win_v, wsem.at[4])
    cp_wsp = pltpu.make_async_copy(wsp_hbm, wsp_v, wsem.at[5])
    cp_wout = pltpu.make_async_copy(wout_hbm, wout_v, wsem.at[6])
    cp_c = pltpu.make_async_copy(c_hbm, c_v, wsem.at[7])
    cp_wk = pltpu.make_async_copy(wkt_hbm, wt_v.at[0:DH], wsem.at[8])
    cp_wv = pltpu.make_async_copy(wvt_hbm, wt_v.at[DH:2 * DH], wsem.at[9])
    cp_bsp = pltpu.make_async_copy(bsp_hbm, bsp_v, wsem.at[10])

    x_copy(0).start()
    cp_c.start()
    cp_wk.start()
    cp_wv.start()

    def norm1(i):
        return _ln(x_v[i * RB:(i + 1) * RB, :].astype(f32))

    def wq_t(k):
        cols = slice(k * (D // 2), (k + 1) * (D // 2))
        wt_v[2 * DH + k * (D // 2):2 * DH + (k + 1) * (D // 2), :] = wq_v[:, cols].astype(f32).T.astype(bf16)

    cp_c.wait()
    cp_ca.start()
    c = c_v[...].astype(f32)
    sc = jnp.broadcast_to(c * jax.nn.sigmoid(c), (16, D)).astype(bf16)
    x_copy(0).wait()
    cp_sa.start()
    n0 = norm1(0)
    cp_ca.wait()
    cp_wq[0].start()
    ca1 = 1.0 + _nn(sc, wmod_v[:, D:2 * D])[0:1]
    cp_sa.wait()
    cp_wq[1].start()
    sa = _nn(sc, wmod_v[:, 0:D])[0:1]
    h = (n0 * ca1 + sa).astype(bf16)
    cp_wq[0].wait()
    x_copy(1).start()
    wq_t(0)
    cp_wq[1].wait()
    x_copy(2).start()
    wq_t(1)
    cp_wk.wait()
    cp_wv.wait()
    x_copy(1).wait()
    x_copy(3).start()

    def proj(i, h):
        cols = slice(i * RB, (i + 1) * RB)
        t = _nt(wt_v[...], h)
        kT = t[0:DH]
        kt_v[:, cols] = kT
        kmx = jnp.max(jnp.max(jnp.abs(kT), axis=0, keepdims=True), axis=1, keepdims=True)
        kmx = jnp.maximum(kmx, 1e-30)
        kf = kT * (127.0 * _recip(kmx))
        th = kf + MAGIC
        kh = th - MAGIC
        tr = (kf - kh) * SIG + MAGIC
        tc = kh * (NREP / SIG) + MAGIC
        k8_v[cols, :] = _low_byte(jnp.concatenate([th] * 6 + [tr, tc], axis=0).T)
        ksc_v[i] = jnp.broadcast_to(kmx * (QK_SCALE / (127.0 * 127.0 * NREP)), (8, 128))
        vT = t[DH:2 * DH]
        vt_v[:, cols] = vT
        qT = t[2 * DH:2 * DH + D]
        qt_v[:, cols] = qT
        q3 = qT.reshape(H, DH, RB)
        if i * RB < AHEAD * TQ:
            q8, qmax = _quant_q(q3[0])
            qc = slice((i * RB) % TQ, (i * RB) % TQ + RB)
            u = (i * RB) // TQ
            q8_v[u, :, qc] = q8
            qsc_v[u, :, qc] = jnp.broadcast_to(qmax, (8, RB))
        q2 = q3 * q3
        qb = jnp.max(q2[:, 0:8] + q2[:, 8:16], axis=0)
        return qb, jnp.sum(kT * kT, axis=0, keepdims=True), jnp.max(jnp.abs(vT), axis=0, keepdims=True)

    stats = None
    for i in range(NRB):
        for g in range(2, len(XG)):
            if XG[g][0] == i + 1:
                x_copy(g).wait()
        hn = (norm1(i + 1) * ca1 + sa).astype(bf16) if i + 1 < NRB else None
        st = proj(i, h)
        stats = st if stats is None else tuple(jnp.maximum(a, b) for a, b in zip(stats, st))
        h = hn

    cp_modb.start()
    cp_wo.start()
    cp_win.start()
    cp_wsp.start()
    cp_wout.start()
    cp_bsp.start()

    qn2max = jnp.max(jnp.sum(stats[0], axis=0, keepdims=True))
    kn2max = jnp.max(stats[1])
    vmx = jnp.max(stats[2])
    safe = jnp.logical_and(qn2max * kn2max <= (LOGIT_BOUND / QK_SCALE) ** 2,
                           jnp.logical_and(vmx <= V_HI, vmx >= V_LO))

    nq = S // TQ
    nk = S // TK

    @pl.when(safe)
    def _attention_fast():
        def body(it, carry):
            chunks = [(u, j) for u in range(NU) for j in range(nk)]
            acc = [None] * NU
            den = [None] * NU
            ps = {}
            itn = jnp.minimum(it + 1, NBODY - 1)

            def rows(i, u):
                return pl.ds(pl.multiple_of((i * (NU // NQ) + u // NQ) * DH, DH), DH)

            def cols(u):
                return slice((u % NQ) * TQ, (u % NQ + 1) * TQ)

            def pv(idx):
                u, j = chunks[idx]
                o = _nn(vt_v[:, j * TK:(j + 1) * TK], ps.pop(idx))
                acc[u] = o if j == 0 else o + acc[u]
                if j == nk - 1:
                    l = jnp.sum(den[u], axis=0, keepdims=True)
                    ot_v[rows(it, u), cols(u)] = acc[u] * (1.0 / l)

            for idx, (u, j) in enumerate(chunks):
                qa = q8_v[u % NSLOT, 0:32, :]
                qb = q8_v[u % NSLOT, 32:64, :]
                qw = jnp.concatenate([qa, qa, qa, qb], axis=0)
                scl = qsc_v[u % NSLOT] * jnp.concatenate([ksc_v[j]] * (TQ // 128), axis=1)
                s = jnp.dot(k8_v[j * TK:(j + 1) * TK, :], qw, preferred_element_type=jnp.int32).astype(f32)
                p = jnp.exp2(s.reshape(TK // 8, 8, TQ) * scl[None])
                d = jnp.sum(p, axis=0)
                den[u] = d if j == 0 else den[u] + d
                ps[idx] = p.reshape(TK, TQ)
                if j % 2 == 0:
                    un = (u + AHEAD) % NU
                    t = j // 2
                    lc = slice(t * 128, (t + 1) * 128)
                    c0 = (un % NQ) * TQ
                    qn = qt_v[rows(it if u + AHEAD < NU else itn, un), c0 + t * 128:c0 + (t + 1) * 128]
                    q8, qmax = _quant_q(qn, jnp.minimum(d[0:1, lc], 1e-30))
                    q8_v[un % NSLOT, :, lc] = q8
                    qsc_v[un % NSLOT, :, lc] = jnp.broadcast_to(qmax, (8, 128))
                if idx >= LAG:
                    pv(idx - LAG)
            for idx in range(len(chunks) - LAG, len(chunks)):
                pv(idx)
            return carry

        lax.fori_loop(0, NBODY, body, 0)

    @pl.when(jnp.logical_not(safe))
    def _attention_exact_max():
        tq = 128
        kb_v[...] = jnp.concatenate([kt_v[...]] * 8, axis=0).T.astype(bf16)

        def body(it, carry):
            hh = it // (S // tq)
            qs = pl.multiple_of((it % (S // tq)) * tq, tq)
            hrows = pl.ds(pl.multiple_of(hh * DH, DH), DH)
            q = qt_v[hrows, pl.ds(qs, tq)].astype(bf16)
            s = _nn(kb_v[...][:, 0:DH], q) * QK_SCALE
            m = jnp.max(s, axis=0, keepdims=True)
            p = jnp.exp2(s - m)
            l = jnp.sum(p, axis=0, keepdims=True)
            o = _nn(vt_v[...], p)
            ot_v[hrows, pl.ds(qs, tq)] = o / l
            return carry

        lax.fori_loop(0, H * (S // tq), body, 0)

    cp_modb.wait()
    mod_v[...] = _nn(sc, wmod_v[:, 2 * D:6 * D])[0:8]
    cp_wo.wait()
    cp_win.wait()

    def phase3(i, carry):
        ga = mod_v[0:1, 0:D]
        sb = mod_v[0:1, D:2 * D]
        cb1 = 1.0 + mod_v[0:1, 2 * D:3 * D]
        rows = [pl.ds(pl.multiple_of((i * P3 + k) * RB, RB), RB) for k in range(P3)]
        hs = []
        for r in rows:
            o = ot_v[:, r].T.astype(bf16)
            x1 = x_v[r, :].astype(f32) + ga * _nn(o, wo_v[...])
            x1_v[r, :] = x1
            hs.append((_ln(x1) * cb1 + sb).astype(bf16))
        for r, h2 in zip(rows, hs):
            z2_v[r, :] = _ln(_gelu_tanh(_nn(h2, win_v[:, FH:F]))).astype(bf16)
            z1_v[r, :] = _gelu_tanh(_nn(h2, win_v[:, 0:FH]))
        return carry

    lax.fori_loop(0, NRB // P3, phase3, 0)

    cp_wsp.wait()
    cp_wout.wait()
    cp_bsp.wait()
    mod_b[...] = bsp_v[...].astype(f32)

    def phase4(i, carry):
        rows = pl.ds(pl.multiple_of(i * RB, RB), RB)
        g = _nn(wsp_v[rows, :], z2_v[...])
        bc = jnp.concatenate(
            [jnp.broadcast_to(mod_b[pl.ds(i * (RB // 128) + k, 1), :], (128, 128)).T for k in range(RB // 128)],
            axis=0)
        g = g + jnp.concatenate([bc] * (FH // 128), axis=1)
        u = (z1_v[rows, :] * g).astype(bf16)
        y = _nn(u, wout_v[...])
        gb = mod_v[0:1, 3 * D:4 * D]
        out_v[rows, :] = (x1_v[rows, :] + gb * y).astype(bf16)
        out_copy(i).start()
        return carry

    lax.fori_loop(0, NRB, phase4, 0)
    for i in range(NRB):
        out_copy(i).wait()


@jax.jit
def pallas_adaLN_cond__grouped_kv_mqa__mixer_gmlp__prompt_kernel(
    A_x: jax.Array,
    A_wq: jax.Array,
    A_wk: jax.Array,
    A_wv: jax.Array,
    A_wo: jax.Array,
    B_x: jax.Array,
    B_w_in: jax.Array,
    B_w_sp: jax.Array,
    B_b_sp: jax.Array,
    B_w_out: jax.Array,
    c: jax.Array,
    w_mod: jax.Array,
):
    del B_x
    hbm = pl.BlockSpec(memory_space=pl.ANY)
    scratch = [
        pltpu.VMEM((S, D), bf16),
        pltpu.VMEM((D, D), bf16),
        pltpu.VMEM((D, D), bf16),
        pltpu.VMEM((D, F), bf16),
        pltpu.VMEM((S, S), bf16),
        pltpu.VMEM((FH, D), bf16),
        pltpu.VMEM((D, 6 * D), bf16),
        pltpu.VMEM((1, D), bf16),
        pltpu.VMEM((S // 128, 128), bf16),
        pltpu.VMEM((8, 4 * D), f32),
        pltpu.VMEM((S // 128, 128), f32),
        pltpu.VMEM((D + 2 * DH, D), bf16),
        pltpu.VMEM((NSLOT, 64, TQ), jnp.int8),
        pltpu.VMEM((NSLOT, 8, TQ), f32),
        pltpu.VMEM((DH, S), f32),
        pltpu.VMEM((S, 128), bf16),
        pltpu.VMEM((S, 128), jnp.int8),
        pltpu.VMEM((NRB, 8, 128), f32),
        pltpu.VMEM((DH, S), f32),
        pltpu.VMEM((D, S), f32),
        pltpu.VMEM((D, S), f32),
        pltpu.VMEM((S, D), f32),
        pltpu.VMEM((S, FH), f32),
        pltpu.VMEM((S, FH), bf16),
        pltpu.VMEM((S, D), bf16),
        pltpu.SemaphoreType.DMA((len(XG),)),
        pltpu.SemaphoreType.DMA((13,)),
        pltpu.SemaphoreType.DMA((NRB,)),
    ]
    out = pl.pallas_call(
        _kernel,
        out_shape=jax.ShapeDtypeStruct((S, D), bf16),
        in_specs=[hbm] * 11,
        out_specs=hbm,
        scratch_shapes=scratch,
        compiler_params=pltpu.CompilerParams(vmem_limit_bytes=100 * 1024 * 1024),
    )(A_x.reshape(S, D), A_wq, A_wk.T, A_wv.T, A_wo, B_w_in, B_w_sp, B_b_sp.reshape(S // 128, 128), B_w_out, c, w_mod)
    return out.reshape(1, S, D)
```

```python
import jax
import jax.numpy as jnp
from jax import lax
import jax.experimental.pallas as pl
import jax.experimental.pallas.tpu as pltpu

S = 2048
D = 512
H = 32
DH = 16
F = 1792
FH = F // 2
EPS = 1e-5
LOG2E = 1.4426950408889634
QK_SCALE = (DH ** -0.5) * LOG2E

RB = 256
NRB = S // RB
P3 = 2
TQ = 512
TK = 256
LAG = 1
NU = 16
NQ = S // TQ
NBODY = H * NQ // NU
NSLOT = 4
AHEAD = 2

NREP = 6.0
SIG = 40.0
LOGIT_BOUND = 60.0
V_HI = 2.0 ** 40
V_LO = 2.0 ** -40

f32 = jnp.float32
bf16 = jnp.bfloat16


def _nt(a, b):
    return lax.dot_general(a, b, (((1,), (1,)), ((), ())), preferred_element_type=f32)


def _nn(a, b):
    return jnp.dot(a, b, preferred_element_type=f32)


def _ln(x):
    m = jnp.mean(x, axis=-1, keepdims=True)
    xc = x - m
    v = jnp.mean(xc * xc, axis=-1, keepdims=True)
    return xc * lax.rsqrt(v + EPS)


def _gelu_tanh(hx):
    c0 = 0.7978845608028654
    c1 = 0.044715 * c0
    u = hx * (2.0 * c0 + (8.0 * c1) * (hx * hx))
    return hx + hx * jnp.tanh(u)


MAGIC = 12582912.0


def _low_byte(t):
    return pltpu.bitcast(t, jnp.int32).astype(jnp.int8)


def _recip(x):
    r = pl.reciprocal(x, approx=True)
    return r * (2.0 - x * r)


def _quant_q(q3, eps=1e-30):
    qmax = jnp.maximum(jnp.max(jnp.abs(q3), axis=-2, keepdims=True), eps)
    qf = q3 * (127.0 * _recip(qmax))
    th = qf + MAGIC
    tr = (qf - (th - MAGIC)) * SIG + MAGIC
    tc = qf * (NREP / SIG) + MAGIC
    return _low_byte(jnp.concatenate([th, th, tc, tr], axis=-2)), qmax


XG = [(0, 1), (1, 2), (2, 4), (4, 8)]


def _kernel(x_hbm, wq_hbm, wkt_hbm, wvt_hbm, wo_hbm, win_hbm, wsp_hbm, bsp_hbm, wout_hbm, c_hbm, wmod_hbm,
            out_hbm,
            x_v, wq_v, wo_v, win_v, wsp_v, wout_v, wmod_v, c_v, bsp_v,
            mod_v, mod_b, wt_v,
            q8_v, qsc_v, kt_v, kb_v, k8_v, ksc_v, vt_v, qt_v, ot_v,
            x1_v, z1_v, z2_v, out_v, ws_v,
            xsem, wsem, osem):
    def x_copy(g):
        r = pl.ds(XG[g][0] * RB, (XG[g][1] - XG[g][0]) * RB)
        return pltpu.make_async_copy(x_hbm.at[r], x_v.at[r], xsem.at[g])

    def out_copy(i):
        r = pl.ds(pl.multiple_of(i * RB, RB), RB)
        return pltpu.make_async_copy(out_v.at[r], out_hbm.at[r], osem.at[i])

    cp_sa = pltpu.make_async_copy(wmod_hbm.at[:, 0:D], wmod_v.at[:, 0:D], wsem.at[0])
    cp_ca = pltpu.make_async_copy(wmod_hbm.at[:, D:2 * D], wmod_v.at[:, D:2 * D], wsem.at[11])
    cp_wq = [pltpu.make_async_copy(wq_hbm.at[:, k * (D // 2):(k + 1) * (D // 2)],
                                   wq_v.at[:, k * (D // 2):(k + 1) * (D // 2)], wsem.at[(1, 12)[k]]) for k in range(2)]
    cp_modb = pltpu.make_async_copy(wmod_hbm.at[:, 2 * D:6 * D], wmod_v.at[:, 2 * D:6 * D], wsem.at[2])
    cp_wo = pltpu.make_async_copy(wo_hbm, wo_v, wsem.at[3])
    cp_win = pltpu.make_async_copy(win_hbm, win_v, wsem.at[4])
    cp_wsp = pltpu.make_async_copy(wsp_hbm, wsp_v, wsem.at[5])
    cp_wout = pltpu.make_async_copy(wout_hbm, wout_v, wsem.at[6])
    cp_c = pltpu.make_async_copy(c_hbm, c_v, wsem.at[7])
    cp_wk = pltpu.make_async_copy(wkt_hbm, wt_v.at[0:DH], wsem.at[8])
    cp_wv = pltpu.make_async_copy(wvt_hbm, wt_v.at[DH:2 * DH], wsem.at[9])
    cp_bsp = pltpu.make_async_copy(bsp_hbm, bsp_v, wsem.at[10])

    x_copy(0).start()
    cp_c.start()
    cp_wk.start()
    cp_wv.start()

    def norm1(i):
        return _ln(x_v[i * RB:(i + 1) * RB, :].astype(f32))

    def wq_t(k):
        cols = slice(k * (D // 2), (k + 1) * (D // 2))
        wt_v[2 * DH + k * (D // 2):2 * DH + (k + 1) * (D // 2), :] = wq_v[:, cols].astype(f32).T.astype(bf16)

    cp_c.wait()
    cp_ca.start()
    c = c_v[...].astype(f32)
    sc = jnp.broadcast_to(c * jax.nn.sigmoid(c), (16, D)).astype(bf16)
    x_copy(0).wait()
    cp_sa.start()
    n0 = norm1(0)
    cp_ca.wait()
    cp_wq[0].start()
    ca1 = 1.0 + _nn(sc, wmod_v[:, D:2 * D])[0:1]
    cp_sa.wait()
    cp_wq[1].start()
    sa = _nn(sc, wmod_v[:, 0:D])[0:1]
    h = (n0 * ca1 + sa).astype(bf16)
    cp_wq[0].wait()
    x_copy(1).start()
    wq_t(0)
    cp_wq[1].wait()
    x_copy(2).start()
    wq_t(1)
    cp_wk.wait()
    cp_wv.wait()
    x_copy(1).wait()
    x_copy(3).start()

    def proj(i, h):
        cols = slice(i * RB, (i + 1) * RB)
        t = _nt(wt_v[...], h)
        kT = t[0:DH]
        kt_v[:, cols] = kT
        kmx = jnp.max(jnp.max(jnp.abs(kT), axis=0, keepdims=True), axis=1, keepdims=True)
        kmx = jnp.maximum(kmx, 1e-30)
        kf = kT * (127.0 * _recip(kmx))
        th = kf + MAGIC
        kh = th - MAGIC
        tr = (kf - kh) * SIG + MAGIC
        tc = kh * (NREP / SIG) + MAGIC
        k8_v[cols, :] = _low_byte(jnp.concatenate([th] * 6 + [tr, tc], axis=0).T)
        ksc_v[i] = jnp.broadcast_to(kmx * (QK_SCALE / (127.0 * 127.0 * NREP)), (8, 128))
        vT = t[DH:2 * DH]
        vt_v[:, cols] = vT
        qT = t[2 * DH:2 * DH + D]
        qt_v[:, cols] = qT
        q3 = qT.reshape(H, DH, RB)
        if i * RB < AHEAD * TQ:
            q8, qmax = _quant_q(q3[0])
            qc = slice((i * RB) % TQ, (i * RB) % TQ + RB)
            u = (i * RB) // TQ
            q8_v[u, :, qc] = q8
            qsc_v[u, :, qc] = jnp.broadcast_to(qmax, (8, RB))
        q2 = q3 * q3
        qb = jnp.max(q2[:, 0:8] + q2[:, 8:16], axis=0)
        return qb, jnp.sum(kT * kT, axis=0, keepdims=True), jnp.max(jnp.abs(vT), axis=0, keepdims=True)

    stats = None
    for i in range(NRB):
        for g in range(2, len(XG)):
            if XG[g][0] == i + 1:
                x_copy(g).wait()
        hn = (norm1(i + 1) * ca1 + sa).astype(bf16) if i + 1 < NRB else None
        st = proj(i, h)
        stats = st if stats is None else tuple(jnp.maximum(a, b) for a, b in zip(stats, st))
        h = hn

    cp_modb.start()
    cp_wo.start()
    cp_win.start()
    cp_wsp.start()
    cp_wout.start()
    cp_bsp.start()

    qn2max = jnp.max(jnp.sum(stats[0], axis=0, keepdims=True))
    kn2max = jnp.max(stats[1])
    vmx = jnp.max(stats[2])
    safe = jnp.logical_and(qn2max * kn2max <= (LOGIT_BOUND / QK_SCALE) ** 2,
                           jnp.logical_and(vmx <= V_HI, vmx >= V_LO))

    nq = S // TQ
    nk = S // TK

    @pl.when(safe)
    def _attention_fast():
        def body(it, carry):
            chunks = [(u, j) for u in range(NU) for j in range(nk)]
            acc = [None] * NU
            den = [None] * NU
            ps = {}
            itn = jnp.minimum(it + 1, NBODY - 1)

            def rows(i, u):
                return pl.ds(pl.multiple_of((i * (NU // NQ) + u // NQ) * DH, DH), DH)

            def cols(u):
                return slice((u % NQ) * TQ, (u % NQ + 1) * TQ)

            def pv(idx):
                u, j = chunks[idx]
                o = _nn(vt_v[:, j * TK:(j + 1) * TK], ps.pop(idx))
                acc[u] = o if j == 0 else o + acc[u]
                if j == nk - 1:
                    l = jnp.sum(den[u], axis=0, keepdims=True)
                    ot_v[rows(it, u), cols(u)] = acc[u] * (1.0 / l)

            for idx, (u, j) in enumerate(chunks):
                qa = q8_v[u % NSLOT, 0:32, :]
                qb = q8_v[u % NSLOT, 32:64, :]
                qw = jnp.concatenate([qa, qa, qa, qb], axis=0)
                scl = qsc_v[u % NSLOT] * jnp.concatenate([ksc_v[j]] * (TQ // 128), axis=1)
                s = jnp.dot(k8_v[j * TK:(j + 1) * TK, :], qw, preferred_element_type=jnp.int32).astype(f32)
                p = jnp.exp2(s.reshape(TK // 8, 8, TQ) * scl[None])
                d = jnp.sum(p, axis=0)
                den[u] = d if j == 0 else den[u] + d
                ps[idx] = p.reshape(TK, TQ)
                if j % 2 == 0:
                    un = (u + AHEAD) % NU
                    t = j // 2
                    lc = slice(t * 128, (t + 1) * 128)
                    c0 = (un % NQ) * TQ
                    qn = qt_v[rows(it if u + AHEAD < NU else itn, un), c0 + t * 128:c0 + (t + 1) * 128]
                    q8, qmax = _quant_q(qn, jnp.minimum(d[0:1, lc], 1e-30))
                    q8_v[un % NSLOT, :, lc] = q8
                    qsc_v[un % NSLOT, :, lc] = jnp.broadcast_to(qmax, (8, 128))
                if idx >= LAG:
                    pv(idx - LAG)
            for idx in range(len(chunks) - LAG, len(chunks)):
                pv(idx)
            return carry

        lax.fori_loop(0, NBODY, body, 0)

    @pl.when(jnp.logical_not(safe))
    def _attention_exact_max():
        tq = 128
        kb_v[...] = jnp.concatenate([kt_v[...]] * 8, axis=0).T.astype(bf16)

        def body(it, carry):
            hh = it // (S // tq)
            qs = pl.multiple_of((it % (S // tq)) * tq, tq)
            hrows = pl.ds(pl.multiple_of(hh * DH, DH), DH)
            q = qt_v[hrows, pl.ds(qs, tq)].astype(bf16)
            s = _nn(kb_v[...][:, 0:DH], q) * QK_SCALE
            m = jnp.max(s, axis=0, keepdims=True)
            p = jnp.exp2(s - m)
            l = jnp.sum(p, axis=0, keepdims=True)
            o = _nn(vt_v[...], p)
            ot_v[hrows, pl.ds(qs, tq)] = o / l
            return carry

        lax.fori_loop(0, H * (S // tq), body, 0)

    cp_modb.wait()
    cp_wo.wait()
    cp_win.wait()
    mod_v[...] = _nn(sc, wmod_v[:, 2 * D:6 * D])[0:8]
    HD = D // 2
    for t in range(HD // 16):
        r = slice(t * 16, (t + 1) * 16)
        q = slice(HD + t * 16, HD + (t + 1) * 16)
        b11 = win_v[r, 0:FH].astype(f32)
        b12 = win_v[r, FH:F].astype(f32)
        b21 = win_v[q, 0:FH].astype(f32)
        b22 = win_v[q, FH:F].astype(f32)
        ws_v[0, r] = (b11 + b22).astype(bf16)
        ws_v[1, r] = (b12 - b22).astype(bf16)
        ws_v[2, r] = (b21 - b11).astype(bf16)
        ws_v[3, r] = (b11 + b12).astype(bf16)
        ws_v[4, r] = (b21 + b22).astype(bf16)

    HS = S // 2
    NL, NE = 384, 512
    C_T, C_B, C_D, C_P = 0, NE, 2 * NE, 2 * NE + FH

    def phase3(i, carry):
        ga = mod_v[0:1, 0:D]
        sb = 0.5 * mod_v[0:1, D:2 * D]
        cb1 = 0.5 + 0.5 * mod_v[0:1, 2 * D:3 * D]
        rows = [pl.ds(pl.multiple_of(i * RB + k * HS, RB), RB) for k in range(2)]
        hs = []
        for r in rows:
            o = ot_v[:, r].T.astype(bf16)
            x1 = x_v[r, :].astype(f32) + ga * _nn(o, wo_v[...])
            x1_v[r, :] = x1
            hs.append(_ln(x1) * cb1 + sb)
        a11, a12 = hs[0][:, 0:HD], hs[0][:, HD:D]
        a21, a22 = hs[1][:, 0:HD], hs[1][:, HD:D]
        m3 = _nn(a11.astype(bf16), ws_v[1])
        m5 = _nn((a11 + a12).astype(bf16), win_v[HD:D, FH:F])
        zt = _ln(_gelu_tanh(m3 + m5))
        m1 = _nn((a11 + a22).astype(bf16), ws_v[0])
        m2 = _nn((a21 + a22).astype(bf16), win_v[0:HD, 0:FH])
        m6 = _nn((a21 - a11).astype(bf16), ws_v[3])
        zb = _ln(_gelu_tanh((m1 - m2) + (m3 + m6)))
        m4 = _nn(a22.astype(bf16), ws_v[2])
        z1_v[rows[1], :] = m2 + m4
        m7 = _nn((a12 - a22).astype(bf16), ws_v[4])
        z1_v[rows[0], :] = ((m1 - m5) + m4) + m7
        r = rows[0]
        z2_v[r, C_T:C_T + NE] = zt[:, 0:NE].astype(bf16)
        z2_v[r, C_B:C_B + NE] = zb[:, NL:FH].astype(bf16)
        z2_v[r, C_D:C_D + FH] = (zb - zt).astype(bf16)
        z2_v[r, C_P:C_P + NL] = (zt[:, 0:NL] + zb[:, NE:FH]).astype(bf16)
        z2_v[r, C_P + NL:C_P + 2 * NL] = (zt[:, 0:NL] + zt[:, NE:FH]).astype(bf16)
        z2_v[r, C_P + 2 * NL:C_P + 3 * NL] = (zb[:, 0:NL] + zb[:, NE:FH]).astype(bf16)
        return carry

    lax.fori_loop(0, NRB // 2, phase3, 0)

    cp_wsp.wait()
    cp_wout.wait()
    cp_bsp.wait()
    mod_b[...] = bsp_v[...].astype(f32)

    def phase4(i, carry):
        rt = pl.ds(pl.multiple_of(i * RB, RB), RB)
        rb = pl.ds(pl.multiple_of(i * RB + HS, RB), RB)
        a11 = wsp_v[rt, 0:HS]
        a12 = wsp_v[rt, HS:S]
        a21 = wsp_v[rb, 0:HS]
        a22 = wsp_v[rb, HS:S]
        add = lambda p, q: (p.astype(f32) + q.astype(f32)).astype(bf16)
        sub = lambda p, q: (p.astype(f32) - q.astype(f32)).astype(bf16)
        n3 = _nn(a11, z2_v[:, C_D + NL:C_D + FH])
        m4 = _nn(a22, z2_v[:, C_D:C_D + NE])
        m5 = _nn(add(a11, a12), z2_v[:, C_B:C_B + NE])
        m7 = _nn(sub(a12, a22), z2_v[:, C_P + 2 * NL:C_P + 3 * NL])
        m1 = _nn(add(a11, a22), z2_v[:, C_P:C_P + NL])
        m6 = _nn(sub(a21, a11), z2_v[:, C_P + NL:C_P + 2 * NL])
        m2 = _nn(add(a21, a22), z2_v[:, C_T:C_T + NE])
        gt = jnp.concatenate([(m1 + m4[:, 0:NL]) + (m7 - m5[:, NE - NL:NE]), m5 - n3], axis=1)
        gbt = jnp.concatenate([m2 + m4, (m1 - m2[:, 0:NL]) + (m6 - n3[:, NE - NL:NE])], axis=1)
        gb = mod_v[0:1, 3 * D:4 * D]
        us = []
        for k, (rows, g) in enumerate(((rt, gt), (rb, gbt))):
            blk = i + k * (NRB // 2)
            bc = jnp.concatenate(
                [jnp.broadcast_to(mod_b[pl.ds(blk * (RB // 128) + t, 1), :], (128, 128)).T for t in range(RB // 128)],
                axis=0)
            g = g + jnp.concatenate([bc] * (FH // 128), axis=1)
            us.append(_gelu_tanh(z1_v[rows, :]) * g)
        ut, ub = us
        b11, b12 = wout_v[0:NL, 0:HD], wout_v[0:NL, HD:D]
        b21, b22 = wout_v[NE:FH, 0:HD], wout_v[NE:FH, HD:D]
        wl1, wl2 = wout_v[NL:NE, 0:HD], wout_v[NL:NE, HD:D]
        cat = lambda p, q: jnp.concatenate([p, q], axis=0)
        e = (ub - ut).astype(bf16)
        p3 = _nn(ut[:, 0:NE].astype(bf16), cat(sub(b12, b22), wl2))
        p5 = _nn((ut[:, 0:NL] + ut[:, NE:FH]).astype(bf16), b22)
        p2 = _nn((ub[:, 0:NL] + ub[:, NE:FH]).astype(bf16), b11)
        p4 = _nn(ub[:, NL:FH].astype(bf16), cat(wl1, sub(b21, b11)))
        p1 = _nn((ut[:, 0:NL] + ub[:, NE:FH]).astype(bf16), add(b11, b22))
        p6 = _nn(e[:, 0:NE], cat(add(b11, b12), wl2))
        q7 = _nn(e[:, NL:FH], cat(wl1, add(b21, b22)))
        yt = jnp.concatenate([((p1 - p5) + p4) - q7, p3 + p5], axis=1)
        yb = jnp.concatenate([p2 + p4, ((p1 - p2) + p3) + p6], axis=1)
        out_v[rt, :] = (x1_v[rt, :] + gb * yt).astype(bf16)
        out_v[rb, :] = (x1_v[rb, :] + gb * yb).astype(bf16)
        out_copy(i).start()
        out_copy(i + NRB // 2).start()
        return carry

    lax.fori_loop(0, NRB // 2, phase4, 0)
    for i in range(NRB):
        out_copy(i).wait()


@jax.jit
def pallas_adaLN_cond__grouped_kv_mqa__mixer_gmlp__prompt_kernel(
    A_x: jax.Array,
    A_wq: jax.Array,
    A_wk: jax.Array,
    A_wv: jax.Array,
    A_wo: jax.Array,
    B_x: jax.Array,
    B_w_in: jax.Array,
    B_w_sp: jax.Array,
    B_b_sp: jax.Array,
    B_w_out: jax.Array,
    c: jax.Array,
    w_mod: jax.Array,
):
    del B_x
    hbm = pl.BlockSpec(memory_space=pl.ANY)
    scratch = [
        pltpu.VMEM((S, D), bf16),
        pltpu.VMEM((D, D), bf16),
        pltpu.VMEM((D, D), bf16),
        pltpu.VMEM((D, F), bf16),
        pltpu.VMEM((S, S), bf16),
        pltpu.VMEM((FH, D), bf16),
        pltpu.VMEM((D, 6 * D), bf16),
        pltpu.VMEM((1, D), bf16),
        pltpu.VMEM((S // 128, 128), bf16),
        pltpu.VMEM((8, 4 * D), f32),
        pltpu.VMEM((S // 128, 128), f32),
        pltpu.VMEM((D + 2 * DH, D), bf16),
        pltpu.VMEM((NSLOT, 64, TQ), jnp.int8),
        pltpu.VMEM((NSLOT, 8, TQ), f32),
        pltpu.VMEM((DH, S), f32),
        pltpu.VMEM((S, 128), bf16),
        pltpu.VMEM((S, 128), jnp.int8),
        pltpu.VMEM((NRB, 8, 128), f32),
        pltpu.VMEM((DH, S), f32),
        pltpu.VMEM((D, S), f32),
        pltpu.VMEM((D, S), f32),
        pltpu.VMEM((S, D), f32),
        pltpu.VMEM((S, FH), f32),
        pltpu.VMEM((S // 2, 3072), bf16),
        pltpu.VMEM((S, D), bf16),
        pltpu.VMEM((5, D // 2, FH), bf16),
        pltpu.SemaphoreType.DMA((len(XG),)),
        pltpu.SemaphoreType.DMA((13,)),
        pltpu.SemaphoreType.DMA((NRB,)),
    ]
    out = pl.pallas_call(
        _kernel,
        out_shape=jax.ShapeDtypeStruct((S, D), bf16),
        in_specs=[hbm] * 11,
        out_specs=hbm,
        scratch_shapes=scratch,
        compiler_params=pltpu.CompilerParams(vmem_limit_bytes=100 * 1024 * 1024),
    )(A_x.reshape(S, D), A_wq, A_wk.T, A_wv.T, A_wo, B_w_in, B_w_sp, B_b_sp.reshape(S // 128, 128), B_w_out, c, w_mod)
    return out.reshape(1, S, D)
```

```python
import jax
import jax.numpy as jnp
from jax import lax
import jax.experimental.pallas as pl
import jax.experimental.pallas.tpu as pltpu

S = 2048
D = 512
H = 32
DH = 16
F = 1792
FH = F // 2
EPS = 1e-5
LOG2E = 1.4426950408889634
QK_SCALE = (DH ** -0.5) * LOG2E

RB = 256
NRB = S // RB
P3 = 2
TQ = 512
TK = 256
LAG = 1
NU = 16
NQ = S // TQ
NBODY = H * NQ // NU
NSLOT = 4
AHEAD = 2

NREP = 6.0
SIG = 40.0
LOGIT_BOUND = 60.0
V_HI = 2.0 ** 40
V_LO = 2.0 ** -40

f32 = jnp.float32
bf16 = jnp.bfloat16


def _nt(a, b):
    return lax.dot_general(a, b, (((1,), (1,)), ((), ())), preferred_element_type=f32)


def _nn(a, b):
    return jnp.dot(a, b, preferred_element_type=f32)


def _ln(x):
    m = jnp.mean(x, axis=-1, keepdims=True)
    xc = x - m
    v = jnp.mean(xc * xc, axis=-1, keepdims=True)
    return xc * lax.rsqrt(v + EPS)


def _gelu_tanh(hx):
    c0 = 0.7978845608028654
    c1 = 0.044715 * c0
    u = hx * (2.0 * c0 + (8.0 * c1) * (hx * hx))
    return hx + hx * jnp.tanh(u)


MAGIC = 12582912.0


def _low_byte(t):
    return pltpu.bitcast(t, jnp.int32).astype(jnp.int8)


def _recip(x):
    r = pl.reciprocal(x, approx=True)
    return r * (2.0 - x * r)


def _quant_q(q3, eps=1e-30):
    qmax = jnp.maximum(jnp.max(jnp.abs(q3), axis=-2, keepdims=True), eps)
    qf = q3 * (127.0 * _recip(qmax))
    th = qf + MAGIC
    tr = (qf - (th - MAGIC)) * SIG + MAGIC
    tc = qf * (NREP / SIG) + MAGIC
    return _low_byte(jnp.concatenate([th, th, tc, tr], axis=-2)), qmax


XG = [(0, 1), (1, 2), (2, 4), (4, 8)]


def _kernel(x_hbm, wq_hbm, wkt_hbm, wvt_hbm, wo_hbm, win_hbm, wsp_hbm, bsp_hbm, wout_hbm, c_hbm, wmod_hbm,
            out_hbm,
            x_v, wq_v, wo_v, win_v, wsp_v, wout_v, wmod_v, c_v, bsp_v,
            mod_v, mod_b, wt_v,
            q8_v, qsc_v, kt_v, kb_v, k8_v, ksc_v, vt_v, qt_v, ot_v,
            x1_v, z1_v, z2_v, out_v, ws_v, zn_v,
            sct_v, zs, xsem, wsem, osem):
    def x_copy(g):
        r = pl.ds(XG[g][0] * RB, (XG[g][1] - XG[g][0]) * RB)
        return pltpu.make_async_copy(x_hbm.at[r], x_v.at[r], xsem.at[g])

    def out_copy(i, k, c):
        copies = []
        for t in range(2):
            r = pl.ds(pl.multiple_of(i * 128 + (2 * k + t) * (S // 4), 128), 128)
            cols = pl.ds(c * (D // 2), D // 2)
            copies.append(pltpu.make_async_copy(out_v.at[r, cols], out_hbm.at[r, cols], osem))
        return copies

    cp_sa = pltpu.make_async_copy(wmod_hbm.at[:, 0:D], wmod_v.at[:, 0:D], wsem.at[0])
    cp_ca = pltpu.make_async_copy(wmod_hbm.at[:, D:2 * D], wmod_v.at[:, D:2 * D], wsem.at[11])
    cp_wq = [pltpu.make_async_copy(wq_hbm.at[:, k * (D // 2):(k + 1) * (D // 2)],
                                   wq_v.at[:, k * (D // 2):(k + 1) * (D // 2)], wsem.at[(1, 12)[k]]) for k in range(2)]
    cp_late = [[pltpu.make_async_copy(wmod_hbm.at[:, (2 + 2 * k) * D:(4 + 2 * k) * D],
                                      wmod_v.at[:, (2 + 2 * k) * D:(4 + 2 * k) * D], wsem.at[13 + 3 * k])]
               + [pltpu.make_async_copy(win_hbm.at[(2 * t + k) * 128:(2 * t + k + 1) * 128],
                                        win_v.at[(2 * t + k) * 128:(2 * t + k + 1) * 128], wsem.at[14 + 3 * k + t])
                  for t in range(2)] for k in range(2)]
    cp_wo = pltpu.make_async_copy(wo_hbm, wo_v, wsem.at[3])
    cp_wsp = pltpu.make_async_copy(wsp_hbm, wsp_v, wsem.at[5])
    cp_wout = pltpu.make_async_copy(wout_hbm, wout_v, wsem.at[6])
    cp_c = pltpu.make_async_copy(c_hbm, c_v, wsem.at[7])
    cp_wk = pltpu.make_async_copy(wkt_hbm, wt_v.at[0:DH], wsem.at[8])
    cp_wv = pltpu.make_async_copy(wvt_hbm, wt_v.at[DH:2 * DH], wsem.at[9])
    cp_bsp = pltpu.make_async_copy(bsp_hbm, bsp_v, wsem.at[10])

    x_copy(0).start()
    cp_c.start()
    cp_wk.start()
    cp_wv.start()

    zs[0] = 0
    zn_v[0:2 * RB, :] = jnp.zeros((2 * RB, FH), f32)

    def norm1(i):
        return _ln(x_v[i * RB:(i + 1) * RB, :].astype(f32))

    def wq_t(k):
        cols = slice(k * (D // 2), (k + 1) * (D // 2))
        wt_v[2 * DH + k * (D // 2):2 * DH + (k + 1) * (D // 2), :] = wq_v[:, cols].astype(f32).T.astype(bf16)

    cp_c.wait()
    cp_ca.start()
    c = c_v[...].astype(f32)
    sc = jnp.broadcast_to(c * jax.nn.sigmoid(c), (16, D)).astype(bf16)
    x_copy(0).wait()
    cp_sa.start()
    n0 = norm1(0)
    cp_ca.wait()
    cp_wq[0].start()
    ca1 = 1.0 + _nn(sc, wmod_v[:, D:2 * D])[0:1]
    cp_sa.wait()
    cp_wq[1].start()
    sa = _nn(sc, wmod_v[:, 0:D])[0:1]
    h = (n0 * ca1 + sa).astype(bf16)
    cp_wq[0].wait()
    x_copy(1).start()
    wq_t(0)
    cp_wq[1].wait()
    x_copy(2).start()
    wq_t(1)
    cp_wk.wait()
    cp_wv.wait()
    x_copy(1).wait()
    x_copy(3).start()

    def proj(i, h):
        cols = slice(i * RB, (i + 1) * RB)
        t = _nt(wt_v[...], h)
        kT = t[0:DH]
        kt_v[:, cols] = kT
        kmx = jnp.max(jnp.max(jnp.abs(kT), axis=0, keepdims=True), axis=1, keepdims=True)
        kmx = jnp.maximum(kmx, 1e-30)
        kf = kT * (127.0 * _recip(kmx))
        th = kf + MAGIC
        kh = th - MAGIC
        tr = (kf - kh) * SIG + MAGIC
        tc = kh * (NREP / SIG) + MAGIC
        k8_v[cols, :] = _low_byte(jnp.concatenate([th] * 6 + [tr, tc], axis=0).T)
        ksc_v[i] = jnp.broadcast_to(kmx * (QK_SCALE / (127.0 * 127.0 * NREP)), (8, 128))
        vT = t[DH:2 * DH]
        vt_v[:, cols] = vT
        qT = t[2 * DH:2 * DH + D]
        qt_v[:, cols] = qT
        q3 = qT.reshape(H, DH, RB)
        if i * RB < AHEAD * TQ:
            q8, qmax = _quant_q(q3[0])
            qc = slice((i * RB) % TQ, (i * RB) % TQ + RB)
            u = (i * RB) // TQ
            q8_v[u, :, qc] = q8
            qsc_v[u, :, qc] = jnp.broadcast_to(qmax, (8, RB))
        q2 = q3 * q3
        qb = jnp.max(q2[:, 0:8] + q2[:, 8:16], axis=0)
        return qb, jnp.sum(kT * kT, axis=0, keepdims=True), jnp.max(jnp.abs(vT), axis=0, keepdims=True)

    stats = None
    for i in range(NRB):
        for g in range(2, len(XG)):
            if XG[g][0] == i + 1:
                x_copy(g).wait()
                if g == 2:
                    for cp in cp_late[0]:
                        cp.start()
        hn = (norm1(i + 1) * ca1 + sa).astype(bf16) if i + 1 < NRB else None
        st = proj(i, h)
        stats = st if stats is None else tuple(jnp.maximum(a, b) for a, b in zip(stats, st))
        h = hn

    sct_v[...] = jnp.broadcast_to(sc[0:1].astype(f32), (128, D)).T

    for cp in cp_late[1]:
        cp.start()
    cp_wo.start()
    cp_wsp.start()
    cp_wout.start()
    cp_bsp.start()

    qn2max = jnp.max(jnp.sum(stats[0], axis=0, keepdims=True))
    kn2max = jnp.max(stats[1])
    vmx = jnp.max(stats[2])
    safe = jnp.logical_and(qn2max * kn2max <= (LOGIT_BOUND / QK_SCALE) ** 2,
                           jnp.logical_and(vmx <= V_HI, vmx >= V_LO))

    for cp in cp_late[0]:
        cp.wait()
    HD = D // 2

    def side_work(it):
        @pl.when(it == NBODY // 2)
        def _():
            for cp in cp_late[1]:
                cp.wait()

        def up(w, z):
            if z is not None:
                zz = jnp.concatenate([jnp.concatenate([z] * (w.shape[1] // 128), axis=1)] * (w.shape[0] // 16), axis=0)
                w = pltpu.bitcast(pltpu.bitcast(w, jnp.int32) | zz, bf16)
            return w.astype(f32)

        nc = 4 * D // NBODY
        acc = None
        for t in range(D // 32):
            z = yield
            w = up(wmod_v[t * 32:(t + 1) * 32, pl.ds(pl.multiple_of(2 * D + it * nc, nc), nc)], z)
            w = w * jnp.concatenate([sct_v[t * 32:(t + 1) * 32, :]] * (nc // 128), axis=1)
            w = jnp.sum(w.reshape(4, 8, nc), axis=0)
            acc = w if acc is None else acc + w
        mod_v[:, pl.ds(pl.multiple_of(it * nc, nc), nc)] = jnp.broadcast_to(jnp.sum(acc, axis=0, keepdims=True), (8, nc))
        nr = HD // NBODY
        r = pl.ds(pl.multiple_of(it * nr, nr), nr)
        q = pl.ds(pl.multiple_of(HD + it * nr, nr), nr)
        for t in range(FH // 128):
            z = yield
            cl = slice(t * 128, (t + 1) * 128)
            cr = slice(FH + t * 128, FH + (t + 1) * 128)
            b11, b12, b21, b22 = up(win_v[r, cl], z), up(win_v[r, cr], z), up(win_v[q, cl], z), up(win_v[q, cr], z)
            ws_v[0, r, cl] = (b11 + b22).astype(bf16)
            ws_v[1, r, cl] = (b12 - b22).astype(bf16)
            ws_v[2, r, cl] = (b21 - b11).astype(bf16)
            ws_v[3, r, cl] = (b11 + b12).astype(bf16)
            ws_v[4, r, cl] = (b21 + b22).astype(bf16)
        while True:
            yield

    nk = S // TK

    @pl.when(jnp.logical_not(safe))
    def _attention_exact_max():
        tq = 128

        def keys(j):
            return pl.ds(pl.multiple_of(j * TK, TK), TK)

        def prep(j, carry):
            side = side_work(j)
            for _ in range(D // 32 + FH // 128 + 1):
                next(side)
            kb_v[keys(j), :] = jnp.concatenate([kt_v[:, keys(j)]] * 8, axis=0).T.astype(bf16)
            return carry

        lax.fori_loop(0, nk, prep, 0)

        def body(it, carry):
            hh = it // (S // tq)
            qs = pl.multiple_of((it % (S // tq)) * tq, tq)
            hrows = pl.ds(pl.multiple_of(hh * DH, DH), DH)
            q = qt_v[hrows, pl.ds(qs, tq)].astype(bf16)

            def chunk(j, c):
                m, l, o = c
                s = _nn(kb_v[keys(j), :][:, 0:DH], q) * QK_SCALE
                mn = jnp.maximum(m, jnp.max(s, axis=0, keepdims=True))
                p = jnp.exp2(s - mn)
                al = jnp.exp2(m - mn)
                return mn, al * l + jnp.sum(p, axis=0, keepdims=True), al * o + _nn(vt_v[:, keys(j)], p)

            init = (jnp.full((1, tq), -jnp.inf, f32), jnp.zeros((1, tq), f32), jnp.zeros((DH, tq), f32))
            _, l, o = lax.fori_loop(0, nk, chunk, init)
            ot_v[hrows, pl.ds(qs, tq)] = o / l
            return carry

        lax.fori_loop(0, H * (S // tq), body, 0)

    @pl.when(safe)
    def _attention_fast():
        def body(it, carry):
            side = side_work(it)
            next(side)
            chunks = [(u, j) for u in range(NU) for j in range(nk)]
            acc = [None] * NU
            den = [None] * NU
            ps = {}
            itn = jnp.minimum(it + 1, NBODY - 1)

            def rows(i, u):
                return pl.ds(pl.multiple_of((i * (NU // NQ) + u // NQ) * DH, DH), DH)

            def cols(u):
                return slice((u % NQ) * TQ, (u % NQ + 1) * TQ)

            def pv(idx):
                u, j = chunks[idx]
                o = _nn(vt_v[:, j * TK:(j + 1) * TK], ps.pop(idx))
                acc[u] = o if j == 0 else o + acc[u]
                if j == nk - 1:
                    l = jnp.sum(den[u], axis=0, keepdims=True)
                    ot_v[rows(it, u), cols(u)] = acc[u] * (1.0 / l)

            for idx, (u, j) in enumerate(chunks):
                qa = q8_v[u % NSLOT, 0:32, :]
                qb = q8_v[u % NSLOT, 32:64, :]
                qw = jnp.concatenate([qa, qa, qa, qb], axis=0)
                scl = qsc_v[u % NSLOT] * jnp.concatenate([ksc_v[j]] * (TQ // 128), axis=1)
                s = jnp.dot(k8_v[j * TK:(j + 1) * TK, :], qw, preferred_element_type=jnp.int32).astype(f32)
                p = jnp.exp2(s.reshape(TK // 8, 8, TQ) * scl[None])
                d = jnp.sum(p, axis=0)
                den[u] = d if j == 0 else den[u] + d
                ps[idx] = p.reshape(TK, TQ)
                if j % 2 == 0:
                    un = (u + AHEAD) % NU
                    t = j // 2
                    lc = slice(t * 128, (t + 1) * 128)
                    c0 = (un % NQ) * TQ
                    qn = qt_v[rows(it if u + AHEAD < NU else itn, un), c0 + t * 128:c0 + (t + 1) * 128]
                    q8, qmax = _quant_q(qn, jnp.minimum(d[0:1, lc], 1e-30))
                    q8_v[un % NSLOT, :, lc] = q8
                    qsc_v[un % NSLOT, :, lc] = jnp.broadcast_to(qmax, (8, 128))
                if idx % 4 == 1:
                    side.send(lax.shift_right_logical(pltpu.bitcast(d[:, 0:128], jnp.int32), 31))
                if idx >= LAG:
                    pv(idx - LAG)
            for idx in range(len(chunks) - LAG, len(chunks)):
                pv(idx)
            return carry

        lax.fori_loop(0, NBODY, body, 0)

    cp_wo.wait()
    GR = 128
    QS = S // 4
    NL, NE = 384, 512

    def grp(i, g):
        return pl.ds(pl.multiple_of(i * GR + g * QS, GR), GR)

    def slot(i, k):
        return pl.ds(pl.multiple_of(i * QS + k * RB, RB), RB)

    def split(n):
        return (n // 256) * 128, n - (n // 256) * 128

    def rhs_ops(t, b):
        n = t.shape[1]
        nl, ne = split(n)
        d = b - t
        return [t[:, 0:ne], b[:, nl:n], d, t[:, 0:nl] + b[:, ne:n], t[:, 0:nl] + t[:, ne:n], b[:, 0:nl] + b[:, ne:n]]

    def rhs_cols(n):
        nl, ne = split(n)
        p = 2 * ne + n
        return [(0, ne), (ne, ne), (2 * ne + nl, ne), (2 * ne, ne), (p, nl), (p + nl, nl), (p + 2 * nl, nl)], p + 3 * nl

    def strassen(a11, a12, a21, a22, n, mm):
        nl, ne = split(n)
        n3 = mm(2, a11)
        m4 = mm(3, a22)
        m5 = mm(1, a11 + a12)
        m7 = mm(6, a12 - a22)
        m1 = mm(4, a11 + a22)
        m6 = mm(5, a21 - a11)
        m2 = mm(0, a21 + a22)
        top = jnp.concatenate([(m1 + m4[:, 0:nl]) + (m7 - m5[:, ne - nl:ne]), m5 - n3], axis=1)
        bot = jnp.concatenate([m2 + m4, (m1 - m2[:, 0:nl]) + (m6 - n3[:, ne - nl:ne])], axis=1)
        return top, bot

    W1 = [w for _, w in rhs_cols(FH)[0]]
    OFF = [sum(rhs_cols(w)[1] for w in W1[:k]) for k in range(7)]

    def pinned(x, zl, kt=0):
        if isinstance(zl, tuple):
            for j in range(x.shape[1] // 128):
                x = pinned(x, zl[0].get(zl[1] + str(j)), j)
            return x
        if not zl:
            return x
        z = zl[0].astype(f32)
        for y in zl[1:]:
            z = z + y.astype(f32)
        z = jnp.minimum(jnp.maximum(z, 0.0), 0.0)
        n = z.shape[0]
        top = jnp.concatenate([x[0:n, j * 128:(j + 1) * 128] + z if j == kt else x[0:n, j * 128:(j + 1) * 128]
                               for j in range(x.shape[1] // 128)], axis=1)
        return jnp.concatenate([top, x[n:]], axis=0)

    def build_rhs(r0, gates=None, zb0=4 * QS):
        acc = None
        n = 0
        order = [(t, k) for t in range(GR // 16) for k in (2, 3, 1, 6, 4, 5, 0)]
        if gates is None:
            order = [(t, k) for k in (2, 3, 1, 6, 4, 5, 0) for t in range(GR // 16)]
        for t, k in order:
            def ld(g, c0, c1):
                return zn_v[pl.ds(zb0 + (g * GR + t * 16), 16), c0:c1]

            def l1(gt, gb):
                return [lambda: ld(gt, 0, NE), lambda: ld(gb, NL, FH), lambda: ld(gb, NL, FH) - ld(gt, NL, FH),
                        lambda: ld(gb, 0, NE) - ld(gt, 0, NE), lambda: ld(gt, 0, NL) + ld(gb, NE, FH),
                        lambda: ld(gt, 0, NL) + ld(gt, NE, FH), lambda: ld(gb, 0, NL) + ld(gb, NE, FH)][k]()

            r = pl.ds(r0 + t * 16, 16) if isinstance(r0, int) else pl.ds(pl.multiple_of(r0 + t * 16, 16), 16)
            c0 = OFF[k]
            for y in rhs_ops(l1(0, 2), l1(1, 3)):
                for j in range(y.shape[1] // 128):
                    z2_v[r, c0:c0 + 128] = y[:, j * 128:(j + 1) * 128].astype(bf16)
                    n += 1
                    if gates is not None and n % 16 == 0:
                        ra = pl.multiple_of(r0 + zs[0] * 16, 16)
                        w = pltpu.bitcast(z2_v[pl.ds(ra, 16), OFF[2]:OFF[2] + 128], jnp.int32)
                        acc = w if acc is None else acc | w
                    c0 += 128
        if gates is not None:
            gates['70'] = [acc]

    P3PLAN = ['-', '-', '-', '-', '-', '-', '-', '-']

    def phase3(i, carry):
        G = {}
        zb0 = pl.multiple_of(i * QS, QS)
        build_rhs(((i + 3) % 4) * GR, G, zb0)
        ga = mod_v[0:1, 0:D]
        sb = 0.5 * mod_v[0:1, D:2 * D]
        cb1 = 0.5 + 0.5 * mod_v[0:1, 2 * D:3 * D]
        hs = []
        for k in range(2):
            o = jnp.concatenate([ot_v[:, grp(i, 2 * k + t)].T for t in range(2)], axis=0)
            o = pinned(o, (G, 'ab'[k])).astype(bf16)
            x0 = jnp.concatenate([x_v[grp(i, 2 * k + t), :] for t in range(2)], axis=0)
            x1 = x0.astype(f32) + ga * _nn(o, wo_v[...])
            x1_v[slot(i, k), :] = x1
            hs.append(_ln(x1) * cb1 + sb)
        a11, a12 = hs[0][:, 0:HD], hs[0][:, HD:D]
        a21, a22 = hs[1][:, 0:HD], hs[1][:, HD:D]
        m3 = _nn(pinned(a11, (G, '3')).astype(bf16), ws_v[1])
        m5 = _nn(pinned((a11 + a12), (G, '5')).astype(bf16), win_v[HD:D, FH:F])
        zt = _ln(_gelu_tanh(m3 + m5))
        m1 = _nn(pinned((a11 + a22), (G, '1')).astype(bf16), ws_v[0])
        m2 = _nn(pinned((a21 + a22), (G, '2')).astype(bf16), win_v[0:HD, 0:FH])
        m6 = _nn(pinned((a21 - a11), (G, '6')).astype(bf16), ws_v[3])
        zb = _ln(_gelu_tanh((m1 - m2) + (m3 + m6)))
        m4 = _nn(pinned(a22, (G, '4')).astype(bf16), ws_v[2])
        z1_v[slot(i, 1), :] = m2 + m4
        m7 = _nn(pinned((a12 - a22), (G, '7')).astype(bf16), ws_v[4])
        z1_v[slot(i, 0), :] = ((m1 - m5) + m4) + m7
        zn_v[pl.ds(zb0 + QS, RB), :] = zt
        zn_v[pl.ds(zb0 + (QS + RB), RB), :] = zb
        return carry

    lax.fori_loop(0, QS // GR, phase3, 0)

    cp_wsp.wait()
    cp_wout.wait()
    cp_bsp.wait()
    mod_b[...] = bsp_v[...].astype(f32)

    ORDER = "m4 n3 m2 m6 m1 m5 p2 p4 m7 q7 p5 p1 p3 p6 y10 y00 y01 y11".split()

    def phase4(i, carry):
        zl = [zn_v[4 * QS + g * GR:4 * QS + (g + 1) * GR, :] for g in range(4)]
        la, lb = [[y[0], y[1], y[2][:, NL:FH], y[2][:, 0:NE]] + y[3:] for y in (rhs_ops(zl[0], zl[2]), rhs_ops(zl[1], zl[3]))]
        add = lambda p, q: (p.astype(f32) + q.astype(f32)).astype(bf16)
        sub = lambda p, q: (p.astype(f32) - q.astype(f32)).astype(bf16)
        cat = lambda p, q: jnp.concatenate([p, q], axis=0)
        hcat = lambda p, q: jnp.concatenate([p, q], axis=1)
        at = cat(wsp_v[grp(i, 0), :], wsp_v[grp(i, 1), :]).astype(f32)
        ab = cat(wsp_v[grp(i, 2), :], wsp_v[grp(i, 3), :]).astype(f32)
        HS = S // 2
        a11, a12, a21, a22 = at[:, 0:HS], at[:, HS:S], ab[:, 0:HS], ab[:, HS:S]

        def mm1(k, a):
            cols = rhs_cols(W1[k])[0]
            wl = jnp.concatenate(rhs_ops(la[k], lb[k]), axis=1)

            def mm2(j, a2):
                c0, w = cols[j]
                return _nn(a2.astype(bf16), cat(z2_v[0:3 * GR, OFF[k] + c0:OFF[k] + c0 + w], wl[:, c0:c0 + w].astype(bf16)))

            return cat(*strassen(a[0:GR, 0:QS], a[0:GR, QS:HS], a[GR:RB, 0:QS], a[GR:RB, QS:HS], W1[k], mm2))

        def gate(k, g, c0):
            bc = cat(*[jnp.broadcast_to(mod_b[pl.ds(i + (2 * k + t) * (QS // GR), 1), :], (128, 128)).T for t in range(2)])
            w = g.shape[1]
            return _gelu_tanh(z1_v[slot(i, k), c0:c0 + w]) * (g + jnp.concatenate([bc] * (w // 128), axis=1))

        b11, b12 = wout_v[0:NL, 0:HD], wout_v[0:NL, HD:D]
        b21, b22 = wout_v[NE:FH, 0:HD], wout_v[NE:FH, HD:D]
        wl1, wl2 = wout_v[NL:NE, 0:HD], wout_v[NL:NE, HD:D]
        MD = NE - NL
        V = {}

        def get(n):
            if n not in V:
                V[n] = rules[n]()
            return V[n]

        rules = {
            'n3': lambda: mm1(2, a11), 'm4': lambda: mm1(3, a22), 'm5': lambda: mm1(1, a11 + a12),
            'm7': lambda: mm1(6, a12 - a22), 'm1': lambda: mm1(4, a11 + a22), 'm6': lambda: mm1(5, a21 - a11),
            'm2': lambda: mm1(0, a21 + a22),
            'tl': lambda: gate(0, ((V['m1'] + V['m4'][:, 0:NL]) - V['m5'][:, MD:NE]) + V['m7'], 0),
            'tr': lambda: gate(0, V['m5'] - V['n3'], NL),
            'bl': lambda: gate(1, V['m2'] + V['m4'], 0),
            'br': lambda: gate(1, ((V['m6'] - V['m2'][:, 0:NL]) - V['n3'][:, MD:NE]) + V['m1'], NE),
            'em': lambda: get('bl')[:, NL:NE] - get('tr')[:, 0:MD],
            'p3': lambda: _nn(hcat(get('tl'), get('tr')[:, 0:MD]).astype(bf16), cat(sub(b12, b22), wl2)),
            'p5': lambda: _nn((get('tl') + get('tr')[:, MD:NE]).astype(bf16), b22),
            'p2': lambda: _nn((get('bl')[:, 0:NL] + get('br')).astype(bf16), b11),
            'p4': lambda: _nn(hcat(get('bl')[:, NL:NE], get('br')).astype(bf16), cat(wl1, sub(b21, b11))),
            'p1': lambda: _nn((get('tl') + get('br')).astype(bf16), add(b11, b22)),
            'p6': lambda: _nn(hcat(get('bl')[:, 0:NL] - get('tl'), get('em')).astype(bf16), cat(add(b11, b12), wl2)),
            'q7': lambda: _nn(hcat(get('em'), get('br') - get('tr')[:, MD:NE]).astype(bf16), cat(wl1, add(b21, b22))),
        }
        gb = mod_v[0:1, 3 * D:4 * D]

        def finish(k, c, y):
            cols = slice(c * HD, (c + 1) * HD)
            res = (x1_v[slot(i, k), cols] + gb[:, cols] * y).astype(bf16)
            for t in range(2):
                out_v[grp(i, 2 * k + t), cols] = res[t * GR:(t + 1) * GR]
            for cp in out_copy(i, k, c):
                cp.start()

        rules.update({
            'y10': lambda: finish(1, 0, V['p2'] + V['p4']),
            'y00': lambda: finish(0, 0, ((V['p4'] - V['q7']) - V['p5']) + V['p1']),
            'y01': lambda: finish(0, 1, V['p5'] + V['p3']),
            'y11': lambda: finish(1, 1, ((V['p1'] - V['p2']) + V['p3']) + V['p6']),
        })
        for n in ORDER:
            get(n)
        return carry

    lax.fori_loop(0, QS // GR, phase4, 0)
    pltpu.make_async_copy(out_v, out_hbm, osem).wait()


@jax.jit
def pallas_adaLN_cond__grouped_kv_mqa__mixer_gmlp__prompt_kernel(
    A_x: jax.Array,
    A_wq: jax.Array,
    A_wk: jax.Array,
    A_wv: jax.Array,
    A_wo: jax.Array,
    B_x: jax.Array,
    B_w_in: jax.Array,
    B_w_sp: jax.Array,
    B_b_sp: jax.Array,
    B_w_out: jax.Array,
    c: jax.Array,
    w_mod: jax.Array,
):
    del B_x
    hbm = pl.BlockSpec(memory_space=pl.ANY)
    scratch = [
        pltpu.VMEM((S, D), bf16),
        pltpu.VMEM((D, D), bf16),
        pltpu.VMEM((D, D), bf16),
        pltpu.VMEM((D, F), bf16),
        pltpu.VMEM((S, S), bf16),
        pltpu.VMEM((FH, D), bf16),
        pltpu.VMEM((D, 6 * D), bf16),
        pltpu.VMEM((1, D), bf16),
        pltpu.VMEM((S // 128, 128), bf16),
        pltpu.VMEM((8, 4 * D), f32),
        pltpu.VMEM((S // 128, 128), f32),
        pltpu.VMEM((D + 2 * DH, D), bf16),
        pltpu.VMEM((NSLOT, 64, TQ), jnp.int8),
        pltpu.VMEM((NSLOT, 8, TQ), f32),
        pltpu.VMEM((DH, S), f32),
        pltpu.VMEM((S, 128), bf16),
        pltpu.VMEM((S, 128), jnp.int8),
        pltpu.VMEM((NRB, 8, 128), f32),
        pltpu.VMEM((DH, S), f32),
        pltpu.VMEM((D, S), f32),
        pltpu.VMEM((D, S), f32),
        pltpu.VMEM((S, D), f32),
        pltpu.VMEM((S, FH), f32),
        pltpu.VMEM((S // 4, 11008), bf16),
        pltpu.VMEM((S, D), bf16),
        pltpu.VMEM((5, D // 2, FH), bf16),
        pltpu.VMEM((10 * RB, FH), f32),
        pltpu.VMEM((D, 128), f32),
        pltpu.SMEM((1,), jnp.int32),
        pltpu.SemaphoreType.DMA((len(XG),)),
        pltpu.SemaphoreType.DMA((19,)),
        pltpu.SemaphoreType.DMA(()),
    ]
    out = pl.pallas_call(
        _kernel,
        out_shape=jax.ShapeDtypeStruct((S, D), bf16),
        in_specs=[hbm] * 11,
        out_specs=hbm,
        scratch_shapes=scratch,
        compiler_params=pltpu.CompilerParams(vmem_limit_bytes=100 * 1024 * 1024),
    )(A_x.reshape(S, D), A_wq, A_wk.T, A_wv.T, A_wo, B_w_in, B_w_sp, B_b_sp.reshape(S // 128, 128), B_w_out, c, w_mod)
    return out.reshape(1, S, D)
```
